```python
import os as _os
_os.environ.setdefault('JAX_PLATFORMS', 'cpu')
import jax
import jax.numpy as jnp

def _softmax(x, axis=-1):
    return jax.nn.softmax(x, axis=axis)

def _gelu(x):
    return jax.nn.gelu(x, approximate=True)

def _silu(x):
    return jax.nn.silu(x)

def _sigmoid(x):
    return jax.nn.sigmoid(x)

def _layernorm(x, axis=-1, eps=1e-05):
    m = jnp.mean(x, axis=axis, keepdims=True)
    v = jnp.var(x, axis=axis, keepdims=True)
    return (x - m) / jnp.sqrt(v + eps)

def _scatter_add(tgt, idx, src, axis=0):
    return tgt.at[idx].add(src)

def _segment_sum(src, seg, n):
    return jax.ops.segment_sum(src, seg, n)

class _Rng:

    def __init__(self, key):
        self._k = key

    def _next(self):
        self._k, sub = jax.random.split(self._k)
        return sub

    def normal(self, shape):
        return jax.random.normal(self._next(), shape, dtype=jnp.bfloat16)

    def randint(self, lo, hi, shape):
        return jax.random.randint(self._next(), shape, lo, hi, dtype=jnp.int32)

    def uniform(self, shape, lo=0.0, hi=1.0):
        return jax.random.uniform(self._next(), shape, jnp.bfloat16, lo, hi)

    def permutation(self, n):
        return jax.random.permutation(self._next(), n)
kernel_name = 'recurrent_scan__spectral_gfnet__mixer_gmlp__prompt'

def setup_inputs():
    _rng = _Rng(jax.random.key(int.from_bytes(__import__("os").urandom(4), "little")))
    _w = lambda a: (lambda t: t.astype(jnp.bfloat16) if jnp.issubdtype(t.dtype, jnp.floating) else t)(jnp.asarray(a))

    def _A_setup():
        B, S, D = (1, 2048, 512)
        Df = D // 2 + 1
        return {'x': _w((lambda *s: _rng.normal(s) * 0.05)(B, S, D)), 'w_r': _w((lambda *s: _rng.normal(s) * 0.1)(S, Df) * 0.02), 'w_i': _w((lambda *s: _rng.normal(s) * 0.1)(S, Df) * 0.02)}
    _A_in = _A_setup()

    def _B_setup():
        B, S, D, F = (1, 2048, 512, 1376)
        Fh = F // 2
        return {'x': _w((lambda *s: _rng.normal(s) * 0.05)(B, S, D)), 'w_in': _w((lambda *s: _rng.normal(s) * 0.4)(D, 2 * Fh)), 'w_sp': _w(0.01 * (lambda *s: _rng.normal(s) * 0.4)(S, S)), 'b_sp': _w(1.0 + 0.01 * (lambda *s: _rng.normal(s) * 0.05)(S)), 'w_out': _w((lambda *s: _rng.normal(s) * 0.05)(Fh, D))}
    _B_in = _B_setup()
    return {'A_x': _A_in['x'], 'A_w_r': _A_in['w_r'], 'A_w_i': _A_in['w_i'], 'B_x': _B_in['x'], 'B_w_in': _B_in['w_in'], 'B_w_sp': _B_in['w_sp'], 'B_b_sp': _B_in['b_sp'], 'B_w_out': _B_in['w_out']}

def reference(A_x, A_w_r, A_w_i, B_x, B_w_in, B_w_sp, B_b_sp, B_w_out):

    def _A_ref(x, w_r, w_i):
        B, S, D = x.shape
        X = (lambda x, axes=(-2, -1): jnp.fft.rfft2(x.astype(jnp.float32), axes=axes))(x, axes=(-2, -1))
        W = w_r + 1j * w_i
        X = X * W
        y = (lambda x, s, axes=(-2, -1): jnp.fft.irfft2(x, s=s, axes=axes).astype(jnp.bfloat16))(X, (S, D), axes=(-2, -1))
        return y

    def _B_ref(x, w_in, w_sp, b_sp, w_out):
        B, S, D = x.shape
        F = w_in.shape[-1]
        Fh = F // 2
        z = _gelu(jnp.einsum('bsd,df->bsf', x, w_in))
        z1 = z[..., :Fh].copy()
        z2 = _layernorm(z[..., Fh:], axis=-1)
        g = jnp.einsum('ts,bsf->btf', w_sp, z2) + b_sp[None, :, None]
        return jnp.einsum('bsf,fd->bsd', z1 * g, w_out)
    x = A_x
    xn = _layernorm(x, axis=-1)
    s = _A_ref(xn, A_w_r, A_w_i)
    g = _silu(_B_ref(xn, B_w_in, B_w_sp, B_b_sp, B_w_out))
    return x + s * g
```

```python
import functools
import math

import numpy as np
import jax
import jax.numpy as jnp
from jax import lax
import jax.experimental.pallas as pl
import jax.experimental.pallas.tpu as pltpu

F32 = jnp.float32
BF16 = jnp.bfloat16
U32 = jnp.uint32
I32 = jnp.int32

S, D, FH = 2048, 512, 688
N1, N2 = 32, 64
EPS = 1e-5
_C0 = math.sqrt(2.0 / math.pi)
ALPHA = (_C0 * 0.044715) ** (1.0 / 3.0)
GC = _C0 / ALPHA
BETA = 0.5 / ALPHA

NT = (((1,), (1,)), ((), ()))


def _pack(m):
    u = np.asarray(m).astype(jnp.bfloat16).view(np.uint16).astype(np.uint32)
    return u[..., 0::2, :] | (u[..., 1::2, :] << 16)


def _constants():
    lane = np.arange(128)
    d = lane - 127.5
    fwd, inv = [], []
    for k in (2 * lane, 2 * lane + 1):
        phi = 2.0 * np.pi * np.outer(d, k) / D
        ck = np.where(k == 0, 1.0, 2.0) / (D * S)
        fwd += [np.cos(phi) / ALPHA, -np.sin(phi) / ALPHA]
        inv += [(np.cos(phi) * ck).T, (-np.sin(phi) * ck).T.copy()]
    inv[1][0, :] = (-1.0) ** lane / (D * S)
    dmat = np.stack(fwd + inv)

    s2 = np.arange(N2)
    k2 = np.arange(N2)
    col = np.arange(2 * N2)
    col_im = (col // 8) % 2
    col_s2 = (col // 16) * 8 + col % 8
    gf, gi = [], []
    for k1 in range(N1):
        g = np.exp(-2j * np.pi * np.outer(k1 + N1 * k2, s2) / S)
        m = np.block([[g.real, -g.imag], [g.imag, g.real]])
        gf.append(m[:, col_im * N2 + col_s2])
        gi.append(m.T)
    gmat = np.stack(gf + gi)

    r = np.arange(16)
    f16 = np.exp(-2j * np.pi * np.outer(r, r) / 16)
    f128 = np.exp(-2j * np.pi * np.outer(lane, lane) / 128)
    nq = np.zeros((5, 128, 128))
    nq[0], nq[1] = f128.real / ALPHA, f128.imag / ALPHA
    nq[2], nq[3] = f128.real, f128.imag
    m = np.block([[f16.real, -f16.imag], [f16.imag, f16.real]])
    nq[4, 0:32, 0:32] = m
    nq[4, 32:64, 0:32] = m.T
    tw = np.exp(-2j * np.pi * np.outer(r, lane) / S)
    tw = np.concatenate([tw.real, tw.imag]).astype(np.float32)
    return _pack(dmat), _pack(gmat), _pack(nq), tw


def _as_bf16(v):
    return pltpu.bitcast(v, BF16)


def _as_u32(v):
    return pltpu.bitcast(v.astype(BF16), U32)


def _cmul_const(z, num, den, sign):
    re, im = z
    num %= den
    if sign < 0:
        num = (den - num) % den
    if num == 0:
        return re, im
    if 4 * num == den:
        return -im, re
    if 2 * num == den:
        return -re, -im
    if 4 * num == 3 * den:
        return im, -re
    c = math.cos(2.0 * math.pi * num / den)
    s = math.sin(2.0 * math.pi * num / den)
    if (8 * num) % den == 0:
        if c * s > 0:
            return (re - im) * c, (re + im) * c
        return (re + im) * c, (im - re) * c
    return re * c - im * s, re * s + im * c


def _dft4(z, sign):
    (ar, ai), (br, bi), (cr, ci), (dr, di) = z
    pr, pi_, qr, qi = ar + cr, ai + ci, ar - cr, ai - ci
    rr, ri, tr, ti = br + dr, bi + di, br - dr, bi - di
    o1 = (qr + ti, qi - tr)
    o3 = (qr - ti, qi + tr)
    if sign > 0:
        o1, o3 = o3, o1
    return [(pr + rr, pi_ + ri), o1, (pr - rr, pi_ - ri), o3]


def _dft8(z, sign):
    ev = _dft4(z[0::2], sign)
    od = _dft4(z[1::2], sign)
    out = [None] * 8
    for j in range(4):
        er, ei = ev[j]
        if j == 2:
            tr, ti = od[j]
            lo, hi = (er + ti, ei - tr), (er - ti, ei + tr)
            if sign > 0:
                lo, hi = hi, lo
        else:
            tr, ti = _cmul_const(od[j], j, 8, sign)
            lo, hi = (er + tr, ei + ti), (er - tr, ei - ti)
        out[j], out[j + 4] = lo, hi
    return out


def _gelu_core(u):
    return u + u * jnp.tanh(u * (GC + u * u))


def _rev_lanes(v):
    idx = 127 - lax.broadcasted_iota(I32, v.shape, 1)
    return jnp.take_along_axis(v, idx, axis=1)


SB = 256
TB = 256
OB = 256


def _kernel(x_hbm, wr_hbm, wi_hbm, win_hbm, wsp_hbm, b_hbm, wout_hbm,
            dmat_hbm, gmat_hbm, nq_hbm, tw_hbm, o_hbm,
            x_v, wr_v, wi_v, win_v, wsp_v, b_v, wout_v, dmat_v, gmat_v, nq_v, tw_v,
            wint, woutt, xn_v, z2_v, h_v, zf, ubuf, ybuf, wscr, bcol, o_v,
            sem_x, sem_sp, sem_m, sem_o):
    def cp(src, dst, sem):
        return pltpu.make_async_copy(src, dst, sem)

    def x_cp(i):
        return cp(x_hbm.at[pl.ds(i * SB, SB)], x_v.at[pl.ds(i * SB, SB)], sem_x.at[i])

    def sp_cp(i):
        return cp(wsp_hbm.at[pl.ds(i * TB, TB)], wsp_v.at[pl.ds(i * TB, TB)], sem_sp.at[i])

    def o_cp(i):
        return cp(o_v.at[pl.ds(i * OB, OB)], o_hbm.at[pl.ds(i * OB, OB)], sem_o.at[i])

    misc = [cp(a, b, sem_m.at[i]) for i, (a, b) in enumerate([
        (win_hbm.at[FH:2 * FH], win_v.at[FH:2 * FH]), (win_hbm.at[0:FH], win_v.at[0:FH]),
        (dmat_hbm, dmat_v), (wr_hbm, wr_v), (wi_hbm, wi_v), (b_hbm, b_v),
        (gmat_hbm, gmat_v), (nq_hbm, nq_v), (tw_hbm, tw_v), (wout_hbm, wout_v)])]
    c_win2, c_win1, c_dmat, c_wr, c_wi, c_b, c_gmat, c_nq, c_tw, c_wout = misc

    x_cp(0).start()
    c_dmat.start()
    c_win2.start()
    for i in range(1, S // SB):
        x_cp(i).start()
    c_win1.start()
    c_b.start()
    sp_cp(0).start()
    sp_cp(1).start()
    for c in (c_wr, c_wi, c_gmat, c_nq, c_tw):
        c.start()
    for i in range(2, S // TB):
        sp_cp(i).start()
    c_wout.start()

    lane = lax.broadcasted_iota(I32, (1, 128), 1)
    alt = jnp.where(lane % 2 == 0, 1.0, -1.0).astype(F32)

    bcol[...] = jnp.zeros(bcol.shape, F32)
    c_dmat.wait()
    c_win2.wait()
    wint[FH // 2:FH, :] = pltpu.bitcast(win_v[FH:2 * FH, :], U32)

    def phase1(i, carry):
        x_cp(i).wait()
        r0 = pl.multiple_of(i * SB, SB)
        x = x_v[pl.ds(r0, SB), :].astype(F32)
        xc = x - jnp.sum(x, axis=1, keepdims=True) * (1.0 / D)
        var = jnp.sum(xc * xc, axis=1, keepdims=True) * (1.0 / D)
        xn = xc * (lax.rsqrt(var + EPS) * ALPHA)
        xb = xn.astype(BF16)
        xn_v[pl.ds(pl.multiple_of(i * (SB // 2), SB // 2), SB // 2), :] = pltpu.bitcast(xb, U32)
        x0, x1, x2, x3 = (xn[:, 128 * j:128 * (j + 1)] for j in range(4))
        lo0, lo1 = x0 + x2, x0 - x2
        hi0, hi1 = _rev_lanes(x1 + x3), _rev_lanes(x1 - x3)
        o0 = lo0 - hi0
        parts = (lo0 + hi0, o0, lo1 + hi1, lo1 - hi1)
        for j in range(4):
            zf[j, pl.ds(r0, SB), :] = jnp.dot(parts[j].astype(BF16), _as_bf16(dmat_v[j]),
                                              preferred_element_type=F32)
        nyq = jnp.sum(o0 * alt, axis=1, keepdims=True)
        acc = bcol[...]
        for j in range(SB // 16):
            acc = jnp.where(lane == i * (SB // 16) + j, nyq[16 * j:16 * (j + 1)], acc)
        bcol[...] = acc

        g = _gelu_core(lax.dot_general(_as_bf16(wint[FH // 2:FH, :]), xb, NT,
                                       preferred_element_type=F32))
        m = jnp.sum(g, axis=0, keepdims=True) * (1.0 / FH)
        v = jnp.maximum(jnp.sum(g * g, axis=0, keepdims=True) * (1.0 / FH) - m * m, 0.0)
        r = lax.rsqrt(v + EPS / BETA ** 2) * (0.5 * BETA)
        z2_v[:, pl.ds(r0, SB)] = _as_u32((g - m) * r)
        return carry

    lax.fori_loop(0, S // SB, phase1, 0)

    def w_prep(j):
        for c, ref in enumerate((wr_v, wi_v)):
            t = pltpu.bitcast(ref[0:256, 128 * j:128 * (j + 1)], U32).T
            for q in range(4):
                row = 33 * (4 * j + q)
                wscr[c, row:row + 32, :] = t[32 * q:32 * (q + 1)]

    def fft_fwd(g, p):
        def ld(s1):
            rows = pl.ds(N2 * s1 + 8 * g, 8)
            return zf[2 * p, rows, :], zf[2 * p + 1, rows, :]
        for b in range(8):
            t = _dft4([ld(8 * a + b) for a in range(4)], -1)
            for c in range(4):
                re, im = _cmul_const(t[c], b * c, 32, -1)
                rows = pl.ds(N2 * (8 * c + b) + 8 * g, 8)
                zf[2 * p, rows, :] = re
                zf[2 * p + 1, rows, :] = im
        for c in range(4):
            t = _dft8([ld(8 * c + b) for b in range(8)], -1)
            for e in range(8):
                ubuf[c + 4 * e, pl.ds(8 * g, 8), 128 * p:128 * (p + 1)] = _as_u32(
                    jnp.concatenate(t[e], axis=0))

    def spectral(k1):
        w = [wscr[c, pl.ds(k1, N2, stride=33), :] for c in range(2)]
        w_re, w_im = (jnp.concatenate([pltpu.bitcast(a << 16, F32),
                                       pltpu.bitcast(a & jnp.uint32(0xFFFF0000), F32)], axis=1)
                      for a in w)
        xf = jnp.dot(_as_bf16(gmat_v[k1]), _as_bf16(ubuf[k1]), preferred_element_type=F32)
        xr, xi = xf[:N2], xf[N2:]
        y = jnp.concatenate([xr * w_re - xi * w_im, xr * w_im + xi * w_re], axis=0)
        vv = jnp.dot(_as_bf16(gmat_v[N1 + k1]), y.astype(BF16), preferred_element_type=F32)
        rows = pl.ds(N2 * k1, N2)
        for p in range(2):
            zf[2 * p, rows, :] = vv[:N2, 128 * p:128 * (p + 1)]
            zf[2 * p + 1, rows, :] = vv[N2:, 128 * p:128 * (p + 1)]

    def fft_inv(g2, p):
        for g in (2 * g2, 2 * g2 + 1):
            for c in range(4):
                t = _dft8([(zf[2 * p, pl.ds(N2 * (c + 4 * e) + 8 * g, 8), :],
                            zf[2 * p + 1, pl.ds(N2 * (c + 4 * e) + 8 * g, 8), :])
                           for e in range(8)], 1)
                for b in range(8):
                    re, im = _cmul_const(t[b], b * c, 32, 1)
                    rows = pl.ds(N2 * (c + 4 * b) + 8 * g, 8)
                    zf[2 * p, rows, :] = re
                    zf[2 * p + 1, rows, :] = im
        for b in range(8):
            t = _dft4([(zf[2 * p, pl.ds(N2 * (c + 4 * b) + 16 * g2, 16), :],
                        zf[2 * p + 1, pl.ds(N2 * (c + 4 * b) + 16 * g2, 16), :])
                       for c in range(4)], 1)
            for a in range(4):
                rows = pl.ds((N2 * (8 * a + b) + 16 * g2) // 2, 8)
                ybuf[2 * p, rows, :] = _as_u32(t[a][0])
                ybuf[2 * p + 1, rows, :] = _as_u32(t[a][1])

    def nyquist():
        sub = lax.broadcasted_iota(I32, (16, 128), 0)
        wn = []
        for ref in (wr_v, wi_v):
            row = ref[256:257, :].astype(F32)
            acc = jnp.zeros((16, 128), F32)
            for j in range(16):
                acc = jnp.where(sub == j, row[:, 128 * j:128 * (j + 1)], acc)
            wn.append(acc)
        cr, ci = tw_v[0:16, :], tw_v[16:32, :]
        pad = jnp.zeros((96, 128), F32)

        def mm(a, b):
            return jnp.dot(a.astype(BF16), b.astype(BF16), preferred_element_type=F32)
        b = bcol[...]
        tr, ti = mm(b, _as_bf16(nq_v[0])), mm(b, _as_bf16(nq_v[1]))
        xf = mm(_as_bf16(nq_v[4, 0:16, :]),
                jnp.concatenate([tr * cr - ti * ci, tr * ci + ti * cr, pad], axis=0))
        xr, xi = xf[:16], xf[16:]
        u = mm(_as_bf16(nq_v[4, 16:32, :]),
               jnp.concatenate([xr * wn[0] - xi * wn[1], xr * wn[1] + xi * wn[0], pad], axis=0))
        ur, ui = u[:16], u[16:]
        bcol[...] = (mm(ur * cr + ui * ci, _as_bf16(nq_v[2]))
                     + mm(ui * cr - ur * ci, _as_bf16(nq_v[3])))

    def gate(i):
        sp_cp(i).wait()
        t0 = i * TB
        gt = lax.dot_general(_as_bf16(z2_v[...]), wsp_v[pl.ds(t0, TB), :], NT,
                             preferred_element_type=F32)
        bias = jnp.concatenate(
            [b_v[i * (TB // 128) + j:i * (TB // 128) + j + 1, :] for j in range(TB // 128)],
            axis=1).astype(F32) * (0.5 * BETA)
        z1 = _gelu_core(lax.dot_general(_as_bf16(wint[0:FH // 2, :]),
                                        _as_bf16(xn_v[pl.ds(t0 // 2, TB // 2), :]), NT,
                                        preferred_element_type=F32))
        h_v[:, pl.ds(t0, TB)] = _as_u32(z1 * (gt + bias))

    c_b.wait()
    c_win1.wait()
    wint[0:FH // 2, :] = pltpu.bitcast(win_v[0:FH, :], U32)
    gate(0)
    for g in range(8):
        fft_fwd(g, 0)
    c_wr.wait()
    c_wi.wait()
    gate(1)
    for g in range(8):
        fft_fwd(g, 1)
    for j in range(16):
        w_prep(j)
    for c in (c_gmat, c_nq, c_tw):
        c.wait()
    for i in range(4):
        gate(2 + i)
        for k1 in range(8 * i, 8 * i + 8):
            spectral(k1)
    gate(6)
    for g2 in range(4):
        fft_inv(g2, 0)
    nyquist()
    c_wout.wait()
    gate(7)
    for g2 in range(4):
        fft_inv(g2, 1)
    woutt[...] = pltpu.bitcast(wout_v[...].T, U32)

    def phase3(i, carry):
        r0 = pl.multiple_of(i * OB, OB)
        rows = pl.ds(r0, OB)
        prows = pl.ds(pl.multiple_of(i * (OB // 2), OB // 2), OB // 2)
        bt = jnp.dot(_as_bf16(woutt[...]), _as_bf16(h_v[:, rows]), preferred_element_type=F32)
        gate_ = (bt + bt * jnp.tanh(bt)).T
        yb = pltpu.roll(_as_u32(bcol[...]), (128 - i * (OB // 16)) % 128, 1)
        yq = jnp.concatenate([pltpu.roll(yb, (128 - j) % 128, 1) for j in range(OB // 16)], axis=0)
        q0 = jnp.where(lane == 0, yq, ybuf[1, prows, :])
        e0 = jnp.dot(_as_bf16(ybuf[0, prows, :]), _as_bf16(dmat_v[4]), preferred_element_type=F32)
        o0 = jnp.dot(_as_bf16(q0), _as_bf16(dmat_v[5]), preferred_element_type=F32)
        e1 = jnp.dot(_as_bf16(ybuf[2, prows, :]), _as_bf16(dmat_v[6]), preferred_element_type=F32)
        o1 = jnp.dot(_as_bf16(ybuf[3, prows, :]), _as_bf16(dmat_v[7]), preferred_element_type=F32)
        lo0, hi0, lo1, hi1 = e0 + o0, e0 - o0, e1 + o1, e1 - o1
        sp = jnp.concatenate([lo0 + lo1, _rev_lanes(hi0 + hi1),
                              lo0 - lo1, _rev_lanes(hi0 - hi1)], axis=1)
        o_v[rows, :] = (x_v[rows, :].astype(F32) + sp * gate_).astype(BF16)
        o_cp(i).start()
        return carry

    lax.fori_loop(0, S // OB, phase3, 0)
    for i in range(S // OB):
        o_cp(i).wait()


@jax.jit
def pallas_recurrent_scan__spectral_gfnet__mixer_gmlp__prompt_kernel(
    A_x, A_w_r, A_w_i, B_x, B_w_in, B_w_sp, B_b_sp, B_w_out,
):
    del B_x
    consts = _constants()
    args = (A_x.reshape(S, D), A_w_r.T, A_w_i.T, B_w_in.T, B_w_sp, B_b_sp.reshape(16, 128),
            B_w_out, *consts)
    vm = pltpu.VMEM
    scratch = [vm(a.shape, a.dtype) for a in args] + [
        vm((FH, D), U32),
        vm((D // 2, FH), U32),
        vm((S // 2, D), U32),
        vm((FH // 2, S), U32),
        vm((FH // 2, S), U32),
        vm((4, S, 128), F32),
        vm((N1, N2, 256), U32),
        vm((4, S // 2, 128), U32),
        vm((2, 33 * N2, 128), U32),
        vm((16, 128), F32),
        vm((S, D), BF16),
        pltpu.SemaphoreType.DMA((S // SB,)),
        pltpu.SemaphoreType.DMA((S // TB,)),
        pltpu.SemaphoreType.DMA((10,)),
        pltpu.SemaphoreType.DMA((S // OB,)),
    ]
    out = pl.pallas_call(
        _kernel,
        out_shape=jax.ShapeDtypeStruct((S, D), BF16),
        in_specs=[pl.BlockSpec(memory_space=pltpu.HBM)] * len(args),
        out_specs=pl.BlockSpec(memory_space=pltpu.HBM),
        scratch_shapes=scratch,
        compiler_params=pltpu.CompilerParams(vmem_limit_bytes=100 * 2 ** 20),
    )(*args)
    return out.reshape(1, S, D)
```

```python
import functools
import math

import numpy as np
import jax
import jax.numpy as jnp
from jax import lax
import jax.experimental.pallas as pl
import jax.experimental.pallas.tpu as pltpu

F32 = jnp.float32
BF16 = jnp.bfloat16
U32 = jnp.uint32
I32 = jnp.int32
NN = (((1,), (0,)), ((), ()))
NT = (((1,), (1,)), ((), ()))

S, D, FH = 2048, 512, 688
NB = S // 256
F0, F1 = 336, 352
FQ = F1 // 2
EPS = 1e-5

ALPHA = (math.sqrt(2.0 / math.pi) * 0.044715) ** (1.0 / 3.0)
GC = math.sqrt(2.0 / math.pi) / ALPHA
BETA = 0.5 / ALPHA

H_AT = ((6, 2), (7, 1))
TAIL = 'B0 B1 B2 B3 B4 I0 I1 B5 I2 I3 I4 B6 I5 I6 I7 B7'
Z0_AT = ('P', 3, 0)
Z1_AT = ('U', 4, 0)
Z3_AT = ('H', 0, 3, 4)
FOLD_AT = ('H', 0, 6, 0)
MIDDLE = ('H', 0, 1, 0)
LATE = ('Q', 1, 4, 3)
FILTER_AT = ('Q', 2, 0, 4)
WOUT_AT = ('Q', 3, 2, 0)
MARGIN = 340
PIN = 340
W_OPS = 0.5
HOLD_NORM, HOLD_PAIR, HOLD_FOLD, HOLD_WSP = (0, 2), ((0,), (3,)), (0, 1), (0, 3)


def _pack(m):
    u = np.asarray(m).astype(jnp.bfloat16).view(np.uint16).astype(np.uint32)
    return u[..., 0::2, :] | (u[..., 1::2, :] << 16)


def _constants():
    lane = np.arange(128)
    fwd, inv = [], []
    for k in (2 * lane, 2 * lane + 1):
        phi = 2.0 * np.pi * np.outer(lane - 127.5, k) / D
        weight = np.where(k == 0, 1.0, 2.0) / (D * S)
        fwd += [np.cos(phi) / ALPHA, -np.sin(phi) / ALPHA]
        inv += [(np.cos(phi) * weight).T, (-np.sin(phi) * weight).T.copy()]
    inv[1][0, :] = (-1.0) ** lane / (D * S)

    t = np.exp(-2j * np.pi * np.outer(np.arange(1, 8), np.arange(256)).reshape(-1, 1) / S)
    twid = np.concatenate([np.tile(t.real, (1, 128)), np.tile(t.imag, (1, 128))], axis=1)

    r = np.arange(16)
    f16 = np.exp(-2j * np.pi * np.outer(r, r) / 16)
    f128 = np.exp(-2j * np.pi * np.outer(lane, lane) / 128)
    nq = np.zeros((5, 128, 128))
    nq[0], nq[1] = f128.real / ALPHA, f128.imag / ALPHA
    nq[2], nq[3] = f128.real, f128.imag
    m = np.block([[f16.real, -f16.imag], [f16.imag, f16.real]])
    nq[4, 0:32, 0:32] = m
    nq[4, 32:64, 0:32] = m.T
    tw = np.exp(-2j * np.pi * np.outer(r, lane) / S)
    tw = np.concatenate([tw.real, tw.imag])
    return _pack(np.stack(fwd + inv)), twid.astype(np.float32), _pack(nq), tw.astype(np.float32)


def _as_bf16(v):
    return pltpu.bitcast(v, BF16)


def _as_u32(v):
    return pltpu.bitcast(v.astype(BF16), U32)


def _cat0(xs):
    return jnp.concatenate(list(xs), axis=0)


def _cat1(xs):
    return jnp.concatenate(list(xs), axis=1)


def _tiles(v):
    return [v[:, 128 * j:128 * (j + 1)] for j in range(v.shape[1] // 128)]


def _groups(v):
    return [v[8 * g:8 * g + 8] for g in range(v.shape[0] // 8)]


def _rev_lanes(v):
    return jnp.take_along_axis(v, 127 - lax.broadcasted_iota(I32, v.shape, 1), axis=1)


def _gelu_core(u):
    return u + u * jnp.tanh(u * (GC + u * u))


def _rotate(z, num, den, sign):
    re, im = z
    num = (sign * num) % den
    if num == 0:
        return re, im
    if 4 * num == den:
        return -im, re
    if 2 * num == den:
        return -re, -im
    if 4 * num == 3 * den:
        return im, -re
    c = math.cos(2.0 * math.pi * num / den)
    s = math.sin(2.0 * math.pi * num / den)
    if (8 * num) % den == 0:
        if c * s > 0:
            return (re - im) * c, (re + im) * c
        return (re + im) * c, (im - re) * c
    return re * c - im * s, re * s + im * c


def _dft4(z, sign):
    (ar, ai), (br, bi), (cr, ci), (dr, di) = z
    pr, pi, qr, qi = ar + cr, ai + ci, ar - cr, ai - ci
    rr, ri, tr, ti = br + dr, bi + di, br - dr, bi - di
    o1, o3 = (qr + ti, qi - tr), (qr - ti, qi + tr)
    if sign > 0:
        o1, o3 = o3, o1
    return [(pr + rr, pi + ri), o1, (pr - rr, pi - ri), o3]


def _dft8_join(even, odd, j, sign):
    er, ei = even[j]
    if j == 2:
        tr, ti = odd[j]
        lo, hi = (er + ti, ei - tr), (er - ti, ei + tr)
        return (hi, lo) if sign > 0 else (lo, hi)
    tr, ti = _rotate(odd[j], j, 8, sign)
    return (er + tr, ei + ti), (er - tr, ei - ti)


SHORT = (2, 5, 6)


def _lhs_operand(k, a11, a12, a21, a22):
    if k == 0:
        return a21 + a22
    if k == 4:
        return a22
    if a11 is None:
        return {1: a22, 3: a21}.get(k)
    if k == 1:
        return a11 + a22
    if k == 3:
        return a21 - a11
    if k == 5:
        return a11 + a12
    return a11 if k == 2 else a12 - a22


def _rhs_operand(k, b11, b12, b21, b22):
    if k in (0, 5):
        return b22 if k else b11
    if k in (1, 3):
        return b11 + (b22 if k == 1 else b12)
    if k == 2:
        return b12 - b22
    return b21 - b11 if k == 4 else b21 + b22


def _load(ops, stores):
    return ops * W_OPS + stores


def _place(loads, cycles, streams):
    loads = np.array(loads, float)
    cycles = np.array(cycles, float)
    placed = [[] for _ in loads]
    order = sorted(range(len(streams)),
                   key=lambda n: (not streams[n][3], cycles[streams[n][0]:streams[n][1]].sum(), n))
    for n in order:
        first, last, tasks, even = streams[n]
        cost = np.array([c for c, _ in tasks], float)
        span = slice(first, last)
        lo, hi = 0.0, 8.0
        for _ in range(40):
            level = 0.5 * (lo + hi)
            if np.maximum(level * cycles[span] - loads[span], 0.0).sum() < cost.sum():
                lo = level
            else:
                hi = level
        share = np.maximum(hi * cycles[span] - loads[span], 0.0)
        if even:
            share = cycles[span] * (cost.sum() / cycles[span].sum())
        where = first + np.searchsorted(np.cumsum(share), np.cumsum(cost) - 0.5 * cost)
        np.add.at(loads, where, cost)
        for j in np.unique(where):
            mine = [t for t, at in zip(tasks, where) if at == j]
            placed[j] += [((m + 0.5) / len(mine), n, t) for m, t in enumerate(mine)]
    return [[t for _, _, t in sorted(p, key=lambda e: e[:2])] for p in placed]


def _kernel(zero_s, x_hbm, wr_hbm, wi_hbm, win_hbm, wsp_hbm, b_hbm, wout_hbm,
            dmat_hbm, twid_hbm, nq_hbm, tw_hbm, o_hbm,
            x_v, wr_v, wi_v, win_v, wsp_v, b_v, wout_v, dmat_v, twid_v, nq_v, tw_v,
            wis_v, wos_v, xn_v, xs_v, ep_v, act_v, zs_v, ws_v, prod_v, hs_v, gate_v, zf, zp,
            yo_v, wt_v, o_v, sem_i, sem_o):
    P = functools.partial
    zero = zero_s[0]
    sealed = set()

    def fetch(ref, r0, r1, c0=0, c1=None, use=0):
        if (id(ref), use) not in sealed:
            sealed.add((id(ref), use))
            spare = pl.multiple_of(zero + (ref.shape[0] - 8), 8)
            ref[pl.ds(spare, 8), 0:128] = jnp.zeros((8, 128), ref.dtype)
        return ref[r0:r1, c0:c1]

    def part(src, dst, *idx):
        return src.at[idx], dst.at[idx]

    stages = [
        [part(x_hbm, x_v, slice(0, 256))],
        [part(win_hbm, win_v, slice(FH, FH + F0))],
        [part(x_hbm, x_v, slice(256, 512))],
        [part(win_hbm, win_v, slice(FH + F0, 2 * FH))],
        [part(win_hbm, win_v, slice(0, F0))],
        [part(win_hbm, win_v, slice(F0, FH)), part(x_hbm, x_v, slice(512, 768))],
        [part(x_hbm, x_v, slice(768, 1280))],
        [part(x_hbm, x_v, slice(1280, S)), part(wsp_hbm, wsp_v, slice(0, 512), slice(0, 1024))],
        [part(wsp_hbm, wsp_v, slice(0, 512), slice(1024, S)),
         part(wsp_hbm, wsp_v, slice(512, 1024)), (b_hbm, b_v), (dmat_hbm, dmat_v),
         part(wsp_hbm, wsp_v, slice(1024, 1536), slice(0, 1024))],
        [(wr_hbm, wr_v), (wi_hbm, wi_v), (twid_hbm, twid_v), (nq_hbm, nq_v), (tw_hbm, tw_v),
         part(wsp_hbm, wsp_v, slice(1024, 1536), slice(1024, S)),
         part(wsp_hbm, wsp_v, slice(1536, S)), (wout_hbm, wout_v)],
    ]
    for n, stage in enumerate(stages):
        for src, dst in stage:
            pltpu.make_async_copy(src, dst, sem_i.at[n]).start()
    latest = []

    def arrive(n):
        slot = n + after(latest[0], jnp.zeros((8, 128), I32))[0, 0] if latest else n
        for src, dst in stages[n]:
            pltpu.make_async_copy(src, dst, sem_i.at[slot]).wait()

    edges = sorted(list(range(0, S + 1, 128)) + [S - 192, S - 160])
    o_cp = {b: pltpu.make_async_copy(o_v.at[a:b], o_hbm.at[a:b], sem_o)
            for a, b in zip(edges, edges[1:])}

    lane = lax.broadcasted_iota(I32, (1, 128), 1)
    alt = jnp.where(lane % 2 == 0, 1.0, -1.0).astype(F32)
    arrive(0)
    never = jnp.full((8, 128), zero, I32) > 0

    def after(dep, v):
        if dep is None:
            return v
        if v.dtype != dep.dtype:
            dep = pltpu.bitcast(dep, v.dtype)
        return _cat0(jnp.where(never, dep, g) for g in _groups(v))

    def widen(dep, packed, hold=(0,)):
        return _as_bf16(_cat1(after(dep if n in hold else None, t)
                              for n, t in enumerate(_tiles(packed)))).astype(F32)

    def matmuls(pairs, dims, tasks):
        res = [lax.dot_general(_as_bf16(a), _as_bf16(b), dims, preferred_element_type=F32)
               for a, b in pairs]
        slots = [(n, c) for n, (a, _) in enumerate(pairs) for c in range(0, a.shape[1], 128)]
        ends = {m // 4: n for m, (n, c) in enumerate(slots) if c + 128 >= pairs[n][0].shape[1]}
        g = max(res[0].shape[0] - PIN, 0) // 8
        latest[:] = [res[0][8 * g:8 * g + 8]]
        start, total = 0.0, sum(cost for cost, _ in tasks)
        for cost, task in tasks:
            at = -(-len(slots) // 4) * start / total
            r = res[ends[min(k for k in ends if k >= int(at))]]
            g = int((at - int(at)) * (r.shape[0] // 8))
            task(r[8 * g:8 * g + 8])
            start += cost
        return res

    nyq, pre, stat = {}, {}, {}

    def norm_rows(v, dep=None):
        packed = pltpu.bitcast(x_v[16 * v:16 * v + 16, :], U32)
        x0, x1, x2, x3 = _tiles(widen(dep, packed, HOLD_NORM))
        tot = (x0 + x1) + (x2 + x3)
        mean = jnp.sum(tot, axis=1, keepdims=True) * (1.0 / D)
        col = jnp.sum(tot * alt, axis=1, keepdims=True)
        sq = jnp.sum((x0 * x0 + x1 * x1) + (x2 * x2 + x3 * x3), axis=1, keepdims=True)
        var = jnp.maximum(sq * (1.0 / D) - mean * mean, 0.0)
        scale = lax.rsqrt(var + EPS) * ALPHA
        xn = [(a - mean) * scale for a in (x0, x1, x2, x3)]
        xn_v[v // 16][8 * (v % 16):8 * (v % 16) + 8, :] = _as_u32(_cat1(xn))
        col = col * scale
        nyq['x'] = jnp.where(lane == v, col, nyq['x']) if v else jnp.broadcast_to(col, (16, 128))
        return xn[3]

    def xn_operands(i, v, dep):
        a, b = (widen(dep, xn_v[i][r:r + 8, :], HOLD_PAIR[r // 64]) for r in (8 * v, 64 + 8 * v))
        for k in (1, 2, 3, 4, 6):
            xs_v[i - 2][8 * v:8 * v + 8, 256 * k:256 * (k + 1)] = _as_u32(
                _rhs_operand(k, a[:, :256], b[:, :256], a[:, 256:], b[:, 256:]))

    def norm_tasks(i):
        rows = [(_load(72, 6), P(norm_rows, 16 * i + 8 * h + v))
                for v in range(8) for h in range(2)]
        tasks = rows[:4]
        for v in range(8):
            tasks += rows[4 + 2 * v:6 + 2 * v] + [(_load(55, 11), P(xn_operands, i, v))]
        return tasks

    def win_operands(v, dep):
        a, b = (widen(dep, pltpu.bitcast(win_v[r:r + 16, :], U32), HOLD_PAIR[r // FH])
                for r in (16 * v, FH + 16 * v))
        for k in range(7):
            wis_v[8 * v:8 * v + 8, 256 * k:256 * (k + 1)] = _as_u32(
                _lhs_operand(k, a[:, :256], a[:, 256:], b[:, :256], b[:, 256:]))

    def activate(j, r0, u):
        a = _gelu_core(u)
        act_v[j][r0:r0 + u.shape[0], :] = a
        for g in _groups(a):
            stat[j] = (stat[j][0] + g, stat[j][1] + g * g) if j in stat else (g, g * g)
        if r0 + u.shape[0] == FH:
            m = jnp.sum(stat[j][0], axis=0, keepdims=True) * (1.0 / FH)
            v = jnp.sum(stat[j][1], axis=0, keepdims=True) * (1.0 / FH) - m * m
            r = lax.rsqrt(jnp.maximum(v, 0.0) + EPS / BETA ** 2) * (0.5 * BETA)
            stat[j] = (jnp.broadcast_to(m, (8, 128)), jnp.broadcast_to(r, (8, 128)))

    def plain_job(half, j, r0, r1, tasks):
        w = pltpu.bitcast(win_v[FH * half + r0:FH * half + r1, :], U32)
        u, = matmuls([(w, fetch(xn_v[j // 2], 64 * (j % 2), 64 * (j % 2 + 1)))], NT, tasks)
        if half:
            activate(j, r0, u)
        else:
            pre.setdefault(('u', j), []).extend(_groups(u))

    def project_job(i, n, tasks):
        def pair(k, r0=0, r1=FH // 2):
            if k in (0, 5):
                h = k // 5
                rhs = fetch(xn_v[i], 64 * h, 64 * (h + 1), 256 * h, 256 * (h + 1))
            else:
                rhs = fetch(xs_v[i - 2], 0, 64, 256 * k, 256 * (k + 1))
            return fetch(wis_v, r0, r1, 256 * k, 256 * (k + 1)), rhs
        m = pre.setdefault(('m', i), [])
        if n < 3:
            m += matmuls([pair(2 * n), pair(2 * n + 1)], NT, tasks)
        else:
            m.append(_cat0(matmuls([pair(6, 0, F1 // 2), pair(6, F1 // 2)], NT, tasks)))
        if n == 1:
            activate(2 * i + 1, 0, (m[1] - m[0]) + (m[2] + m[3]))
        if n == 2:
            activate(2 * i, 0, m[0] + m[4])

    def linear1(t, w):
        if ('m', t) not in pre:
            return (_cat0(pre['u', j][2 * w:2 * w + 2]) for j in (2 * t, 2 * t + 1))
        m1, m3, m4, m5, m7 = (pre['m', t][k][16 * w:16 * w + 16] for k in (1, 2, 4, 5, 6))
        return (m1 + m4) + (m7 - m5), m3 + m5

    z_order = ((2, (0,)), (4, (3,)), (1, ()), (0, (2,)), (3, ()), (5, (1,)), (6, ()))
    w_order = ((0, (0,)), (5, (3,)), (1, ()), (2, (1,)), (3, ()), (4, (2,)), (6, ()))
    w_plain = ((0, 0), (0, 5), (5, 0), (5, 5))

    def slots_of(order, skip):
        keys = [(k, j) for k, _ in order for j in range(7) if (k, j) not in skip]
        return {key: n for n, key in enumerate(keys)}
    z_slots, w_slots = slots_of(z_order, ()), slots_of(w_order, w_plain)

    def nested_operands(ref, v, source, rule, order, slots):
        state = {'left': ()}

        def step(k, fresh, dep):
            for n in fresh:
                state[n] = source(n, dep)
            blocks = [rule(k, *(state[n][m] if n in state else None for n in range(4)))
                      for m in range(4)]
            if not fresh:
                blocks[3] = _cat0([blocks[3][:8], after(dep, blocks[3][8:])])
            js = [j for j in range(7) if (k, j) in slots]
            ops = [rule(j, *blocks) for j in js]
            ops = tuple(blocks[3] if op is None else op for op in ops)
            n0 = slots[k, js[0]] - len(state['left'])
            ops = state['left'] + ops + (ops[-1:] if k == 6 else ())
            for n in range(0, len(ops) - 1, 2):
                ref[8 * v:8 * v + 8, 128 * (n0 + n):128 * (n0 + n + 2)] = _as_u32(
                    _cat1(ops[n:n + 2]))
            state['left'] = ops[len(ops) // 2 * 2:]
        return [(_load(27 + 14 * len(fresh), 7 + 5 * len(fresh)), P(step, k, fresh))
                for k, fresh in order]

    def z2_tasks(q):
        def source(v, n, dep):
            tiles = (4 * q + n % 2, 4 * q + 2 + n % 2)
            mean = {j: after(dep, stat[j][0]) for j in tiles}

            def normed(j, r):
                if n < 2 and r >= F0:
                    return None
                r += F0 * (n // 2)
                return _cat0((a - mean[j]) * stat[j][1]
                             for a in _groups(fetch(act_v[j], r, r + 16)))
            return [normed(j, r) for r in (FQ + 16 * v, 16 * v) for j in tiles]
        return [t for v in range(FQ // 16) for t in nested_operands(
            zs_v[q], v, P(source, v), _lhs_operand, z_order, z_slots)]

    def wsp_tile(r, c, rows):
        return pltpu.bitcast(wsp_v[r:r + rows, c:c + 128], U32)

    def wsp_tasks(tq, qs):
        def source(q, v, n, dep):
            return [widen(dep if m in HOLD_WSP else None,
                          wsp_tile(512 * tq + 256 * (m % 2) + 128 * (n % 2) + 16 * v,
                                   512 * q + 256 * (m // 2) + 128 * (n // 2), 16))
                    for m in range(4)]
        return [t for q in qs for v in range(8) for t in nested_operands(
            ws_v[4 * (tq % 3) + q], v, P(source, q, v), _rhs_operand, w_order, w_slots)]

    inner = {}

    def height(k, j):
        return FQ - 16 if k in SHORT and j in SHORT else FQ

    def product_job(tq, k, js, qs, tasks):
        def pair(j, r0=0, r1=None):
            c = 128 * z_slots[k, j]
            lhs = _cat1(fetch(zs_v[q], r0, r1 or height(k, j) // 2, c, c + 128) for q in qs)
            if (k, j) in w_plain:
                o = 256 * (j // 5) + 128 * (k // 5)
                return lhs, _cat1(wsp_tile(512 * tq + o, 512 * q + o, 128) for q in qs)
            c = 128 * w_slots[k, j]
            return lhs, _cat1(fetch(ws_v[4 * (tq % 3) + q], 0, 64, c, c + 128, tq) for q in qs)
        if len(js) * len(qs) == 4:
            res = matmuls([pair(j) for j in js], NT, tasks)
        else:
            res = [_cat0(matmuls([pair(js[0], 0, 48), pair(js[0], 48)], NT, tasks))]
        for j, r in zip(js, res):
            inner[tq, k, j] = inner[tq, k, j] + r if (tq, k, j) in inner else r
        if qs[-1] == 3:
            out, n = prod_v[tq], height(k, 2)
            m2, m1, m3, m6, m4, m5, m7 = (inner.get((tq, k, j)) for j in range(7))
            c0, c1 = slice(256 * k, 256 * k + 128), slice(256 * k + 128, 256 * k + 256)
            if 3 in js:
                c22 = (m1 - m2) + m6
                out[0:FQ, c1] = _cat0([c22[:n] + m3, c22[n:]]) if n < FQ else c22 + m3
            if 4 in js:
                out[0:FQ, c0] = m2 + m4
            if 5 in js:
                out[FQ:FQ + n, c1] = m3 + m5
            if 6 in js:
                out[FQ:FQ + n, c0] = (m1[:n] + m4[:n]) + (m7 - m5)

    def gate_tasks(t, v):
        state = {}

        def bias(j, dep):
            b = after(dep, jnp.broadcast_to(b_v[j:j + 1, :].astype(F32) * (0.5 * BETA), (8, 128)))
            return _cat0([b, b])

        def outer(k):
            c = 256 * k + 128 * (t % 2)
            return fetch(prod_v[t // 2], 16 * v, 16 * v + 16, c, c + 128)

        def lower(dep):
            m2, m1, m6, m4 = (outer(k) for k in (0, 1, 3, 4))
            m4 = m4 + bias(2 * t, dep)
            m3 = bias(2 * t + 1, dep)
            if 16 * v < F0:
                m3 = m3 + outer(2)
            z21, z22 = (_gelu_core(after(dep, u)) for u in linear1(t, F0 // 16 + v))
            state['v'] = (m1 + m4, m3, z21 * (m2 + m4), z22 * ((m1 - m2) + (m3 + m6)))

        def upper(dep):
            m14, m3, h21, h22 = state['v']
            if 16 * v < F0:
                m5, m7 = outer(5), outer(6)
                z11, z12 = (_gelu_core(after(dep, u)) for u in linear1(t, v))
                h11, h12 = z11 * (m14 + (m7 - m5)), z12 * (m3 + m5)
                ops = [_rhs_operand(k, h11, h12, h21, h22) for k in range(7)]
            else:
                ops = [h22, h22, h22, h22, h21, h22, h21 + h22]
            hs_v[t][8 * v:8 * v + 8, :] = _as_u32(_cat1(ops + [h22]))
        return [(_load(52, 3), lower), (_load(62, 9), upper)]

    def fold_rows(b, n, dep):
        r = 32 * (b % 4) + 8 * (n // 4)
        x0, x1, x2, x3 = _tiles(widen(dep, fetch(xn_v[2 * (n % 4) + b // 4], r, r + 8), HOLD_FOLD))
        s02, d02, s13, d13 = x0 + x2, x0 - x2, _rev_lanes(x1 + x3), _rev_lanes(x1 - x3)
        ep_v[b][8 * n:8 * n + 8, :] = _as_u32(_cat1([s02 + s13, s02 - s13, d02 + d13, d02 - d13]))

    def get(stage, p, n):
        return tuple(_tiles(fetch(zf[2 * (stage % 2) + p], 8 * n, 8 * n + 8, use=stage)))

    def put(stage, p, n, z):
        zf[2 * (stage % 2) + p][8 * n:8 * n + 8, :] = _cat1(z)

    def dft_job(b, tasks):
        res = matmuls([(fetch(ep_v[b], 0, 128, 128 * j, 128 * (j + 1)), dmat_v[j])
                       for j in range(4)], NN, tasks)
        for g in range(8):
            for p in range(2):
                rows = [64 * (g // 2) + 16 * a + 8 * (g % 2) for a in range(4)]
                t = _dft4([(res[2 * p][r:r + 8], res[2 * p + 1][r:r + 8]) for r in rows], -1)
                for c in range(4):
                    put(0, p, 8 * (8 * c + b) + g, _rotate(t[c], b * c, 32, -1))

    def weight_rows(j, c, dep):
        t = pltpu.bitcast((wr_v, wi_v)[c][0:256, 128 * j:128 * (j + 1)], U32)
        wt_v[128 * j:128 * (j + 1), 128 * c:128 * (c + 1)] = _cat0([after(dep, t[:8]), t[8:]]).T

    def held(dep, z):
        return [(after(dep, z[0][0]), z[0][1])] + z[1:]

    def radix8(source, sink, sign, ops, stores):
        def dft8(dep):
            even, odd = ([source(n) for n in range(h, 8, 2)] for h in range(2))
            even, odd = _dft4(even[:2] + held(dep, even[2:]), sign), _dft4(odd, sign)
            for j in range(4):
                for n, z in zip((j, j + 4), _dft8_join(even, odd, j, sign)):
                    sink(n, z)
        return _load(56 + ops, stores), dft8

    def fwd_b(p, g, c):
        return radix8(lambda b: get(0, p, 8 * (8 * c + b) + g),
                      lambda e, z: put(1, p, 8 * (c + 4 * e) + g,
                                       _rotate(z, (c + 4 * e) * g, 256, -1)), -1, 42, 16)

    def fwd_g(p, k):
        def sink(m, z):
            r = 9 * (k + 32 * m)
            zp[2 * p][r:r + 8, :], zp[2 * p + 1][r:r + 8, :] = z
        return radix8(lambda g: get(1, p, 8 * k + g), sink, -1, 0, 16)

    def filter_tasks(p, w):
        spectrum = {}

        def twiddle(i):
            r = 256 * (i - 1) + 8 * w
            return twid_v[r:r + 8, 0:128], twid_v[r:r + 8, 128:256]

        def source(i):
            re, im = (zp[2 * p + h][pl.ds(72 * w + i, 8, stride=9), :] for h in range(2))
            if i == 0:
                return re, im
            tr, ti = twiddle(i)
            return re * tr - im * ti, re * ti + im * tr

        def weigh(dep):
            arg = after(dep, jnp.full((8, 128), 0xFFFF0000 if p else 16, U32))
            for n in range(8):
                (re, im), r = spectrum[n], 256 * n + 8 * w
                wr, wi = (pltpu.bitcast(u & arg if p else u << arg, F32)
                          for u in _tiles(fetch(wt_v, r, r + 8)))
                spectrum[n] = (re * wr - im * wi, re * wi + im * wr)

        def sink(i, z):
            re, im = z
            if i:
                tr, ti = twiddle(i)
                re, im = re * tr + im * ti, im * tr - re * ti
            rows = pl.ds(72 * w + i, 8, stride=9)
            zp[4 + 2 * p][rows, :], zp[5 + 2 * p][rows, :] = re, im
        return [radix8(source, lambda n, z: spectrum.update({n: z}), -1, 42, 2),
                (_load(65, 2), weigh), radix8(lambda n: spectrum[n], sink, 1, 42, 16)]

    def inv_g(p, k):
        def source(m):
            r = 9 * (k + 32 * m)
            return zp[4 + 2 * p][r:r + 8, :], zp[5 + 2 * p][r:r + 8, :]
        return radix8(source, lambda g, z: put(2, p, 8 * k + g, _rotate(z, k * g, 256, 1)),
                      1, 42, 16)

    def inv_b(p, g, c):
        return radix8(lambda e: get(2, p, 8 * (c + 4 * e) + g),
                      lambda b, z: put(3, p, 8 * (c + 4 * b) + g, _rotate(z, b * c, 32, 1)),
                      1, 29, 16)

    def inv_a(p, g2, b, dep):
        t = [_dft4(held(dep, [get(3, p, 8 * (c + 4 * b) + g) for c in range(4)]), 1)
             for g in (2 * g2, 2 * g2 + 1)]
        r = 32 * (b % 4) + 8 * g2
        for a in range(4):
            yo_v[2 * a + b // 4][r:r + 8, 256 * p:256 * (p + 1)] = _as_u32(
                _cat0([_cat1(t[0][a]), _cat1(t[1][a])]))

    def nyquist():
        def mm(a, b):
            return jnp.dot(a.astype(BF16), b.astype(BF16), preferred_element_type=F32)
        sub = lax.broadcasted_iota(I32, (16, 128), 0)
        cr, ci = tw_v[0:16, :], tw_v[16:32, :]
        pad = jnp.zeros((96, 128), F32)
        tr, ti = mm(nyq['x'], _as_bf16(nq_v[0])), mm(nyq['x'], _as_bf16(nq_v[1]))
        yield
        xf = mm(_as_bf16(nq_v[4, 0:16, :]), _cat0([tr * cr - ti * ci, tr * ci + ti * cr, pad]))
        xr, xi = xf[:16], xf[16:]
        yield
        wn = []
        for ref in (wr_v, wi_v):
            acc = jnp.zeros((16, 128), F32)
            for j, piece in enumerate(_tiles(ref[256:257, :].astype(F32))):
                acc = jnp.where(sub == j, piece, acc)
            wn.append(acc)
        u = mm(_as_bf16(nq_v[4, 16:32, :]),
               _cat0([xr * wn[0] - xi * wn[1], xr * wn[1] + xi * wn[0], pad]))
        ur, ui = u[:16], u[16:]
        yield
        nyq['y'] = _as_u32(mm(ur * cr + ui * ci, _as_bf16(nq_v[2]))
                           + mm(ui * cr - ur * ci, _as_bf16(nq_v[3])))
        yield

    depth = (F0, F1, F0, F0, F1, F1, F1)
    proj = {}

    def wout_operand(k, dep):
        lo = _cat0([wout_v[0:F0, :].astype(F32), jnp.zeros((F1 - F0, D), F32)])
        hi = wout_v[F0:FH, :].astype(F32)
        op = _lhs_operand(k, lo[:, :256], hi[:, :256], lo[:, 256:], hi[:, 256:])
        wos_v[128 * k:128 * (k + 1), 0:depth[k]] = pltpu.bitcast(
            op[0:depth[k]].astype(BF16).T, U32)

    def emit(i, h):
        if ('y', i) not in proj or (i, 6) not in proj:
            return
        for r in range(128 * h, 128 * (h + 1), 16):
            e0, o0, e1, o1 = (a[r:r + 16] for a in proj['y', i])
            lo0, hi0, lo1, hi1 = e0 + o0, e0 - o0, e1 + o1, e1 - o1
            s = _cat1([lo0 + lo1, _rev_lanes(hi0 + hi1), lo0 - lo1, _rev_lanes(hi0 - hi1)])
            g = fetch(gate_v[2 * i + h], r % 128, r % 128 + 16)
            rows = slice(256 * i + r, 256 * i + r + 16)
            o_v[rows, :] = (x_v[rows, :].astype(F32) + s * g).astype(BF16)
            if rows.stop in o_cp:
                o_cp[rows.stop].start()

    def output_job(i, ks, tasks):
        res = matmuls([(fetch(wos_v, 128 * k, 128 * (k + 1), 0, depth[k]),
                        fetch(hs_v[i], 0, depth[k] // 2, 128 * k, 128 * (k + 1))) for k in ks],
                      NN, tasks)
        proj.update({(i, k): r for k, r in zip(ks, res)})

        def keep(h, c, b):
            gate_v[2 * i + h][0:128, 256 * c:256 * (c + 1)] = (b + b * jnp.tanh(b)).T
        m2, m1, m3, m6 = (proj[i, k] for k in range(4))
        if ks[0] == 0:
            keep(1, 1, (m1 - m2) + (m3 + m6))
        else:
            m5, m4, m7 = res
            keep(1, 0, m3 + m5)
            emit(i, 1)
            keep(0, 1, m2 + m4)
            keep(0, 0, (m1 + m4) + (m7 - m5))
            emit(i, 0)

    def inverse_job(i, tasks):
        y = _tiles(fetch(yo_v[i], 0, 128))
        col = _cat0(pltpu.roll(nyq['y'], (128 - v) % 128, 1) for v in range(16 * i, 16 * (i + 1)))
        y[1] = jnp.where(lane == 0, col, y[1])
        proj['y', i] = matmuls([(y[j], dmat_v[4 + j]) for j in range(4)], NN, tasks)
        emit(i, 0)
        emit(i, 1)

    jobs, names, streams = [], {}, []

    def job(name, cycles, load, fn):
        names[name] = len(jobs)
        jobs.append((cycles, load, [], fn, []))

    def half_products(k, qs):
        for js in ((0, 1), (2, 3), (4, 5), (6,)):
            job(('H', qs[0], k, js[0]), 88 * len(js),
                _load(22 + 24 * qs[0], 22 + 3 * qs[0]) * len(js), P(product_job, 0, k, js, qs))

    def stream(first, last, tasks, skip=0, margin=MARGIN, even=False):
        first, last, gap = names[first] + skip, names[last], 0
        while gap < margin and last - 1 > first:
            last -= 1
            gap += jobs[last][0]
        streams.append((first, last, tasks, even))

    for n, (half, r0, r1) in enumerate(((1, 0, F0), (1, F0, FH), (0, 0, F0), (0, F0, FH))):
        for j in range(4):
            job(('P', n, j), r1 - r0, _load(215 + 344 * half, 43), P(plain_job, half, j, r0, r1))
    for i in range(2, NB):
        for n, load in enumerate(((172, 172), (1118, 172), (946, 258), (86, 86))):
            job(('U', i, n), FH if n < 3 else FH // 2, _load(*load), P(project_job, i, n))
            if (i, n) in H_AT:
                half_products(H_AT.index((i, n)), (0, 1))
    for k in range(len(H_AT), 7):
        half_products(k, (0, 1))
    for k in range(7):
        half_products(k, (2, 3))
        job(('D', k), 256, _load(500, 140), P(dft_job, k))
    for tq in range(1, 4):
        for k in range(7):
            for j in range(7):
                job(('Q', tq, k, j), height(k, j), _load(91, 28),
                    P(product_job, tq, k, (j,), range(4)))
            if (tq, k) == (1, 0):
                job(('D', 7), 256, _load(500, 140), P(dft_job, 7))
    for kind, i in ((a, int(b)) for a, b in TAIL.split()):
        if kind == 'B':
            job(('B', i, 0), 768, _load(420, 128), P(output_job, i, (0, 1, 2, 3)))
            job(('B', i, 1), 576, _load(550, 160), P(output_job, i, (5, 4, 6)))
        else:
            job(('I', i), 256, _load(900, 100), P(inverse_job, i))

    for n, name in enumerate((('P', 0, 0), ('P', 0, 2), ('P', 1, 0), ('P', 2, 0), ('P', 2, 3),
                              ('U', 2, 0), ('U', 4, 0), MIDDLE, LATE)):
        jobs[names[name]][2].append(P(arrive, n + 1))
    jobs[names['P', 0, 2]][2].extend(P(norm_rows, v) for v in range(16, 32))
    steps = nyquist()
    for k in range(4):
        jobs[names['Q', 2, k, 3]][4].append(P(next, steps))

    ops = [(_load(66, 15), P(win_operands, v)) for v in range(FH // 16)]
    stream(('P', 2, 0), ('P', 3, 0), ops[:F0 // 16], margin=0)
    stream(('P', 3, 0), ('U', 2, 0), ops[F0 // 16:], margin=1)
    for i in range(2, NB):
        stream(('P', 2, 3) if i == 2 else ('U', i - 1, 0), ('U', i, 0), norm_tasks(i), margin=1)
    for b in range(8):
        stream(('D', b - 1) if b else FOLD_AT, ('D', b),
               [(_load(36, 5), P(fold_rows, b, n)) for n in range(16)], margin=170, even=True)
    stream(Z0_AT, Z1_AT, z2_tasks(0), margin=0)
    stream(Z1_AT, ('H', 0, 0, 0), z2_tasks(1) + wsp_tasks(0, (0, 1)))
    stream(('H', 0, 0, 0), MIDDLE, z2_tasks(2), margin=0)
    stream(MIDDLE, Z3_AT, wsp_tasks(0, (2, 3)), margin=0)
    stream(Z3_AT, ('H', 2, 0, 0), z2_tasks(3))
    stream(('H', 2, 0, 0), ('Q', 1, 0, 0), wsp_tasks(1, range(4)))
    stream(('Q', 1, 0, 0), LATE, wsp_tasks(2, (0, 1)), margin=0)
    stream(LATE, ('Q', 2, 0, 0), wsp_tasks(2, (2, 3)))
    stream(('Q', 2, 0, 0), ('Q', 3, 0, 0), wsp_tasks(3, range(4)))
    for t in range(NB):
        stream(('Q', t // 2, 6, 6) if t > 1 else ('H', 2, 6, 6), ('B', t, 0),
               [task for v in range(F1 // 16) for task in gate_tasks(t, v)], skip=3)
    stream(WOUT_AT, ('B', 0, 0), [(_load(250, 60), P(wout_operand, k)) for k in range(7)],
           even=True)
    grid = [(p, c, n) for p in range(2) for c in range(4) for n in range(8)]
    stream(('D', 7), FILTER_AT,
           [fwd_b(p, g, c) for p, c, g in grid] + [fwd_g(p, c + 4 * e) for p, c, e in grid],
           skip=1, margin=0)
    stream(LATE, FILTER_AT,
           [(_load(18, 16), P(weight_rows, j, c)) for j in range(16) for c in range(2)], even=True)
    stream(FILTER_AT, ('I', 0),
           [task for p, c, n in grid for task in filter_tasks(p, 8 * c + n)]
           + [inv_g(p, c + 4 * e) for p, c, e in grid] + [inv_b(p, g, c) for p, c, g in grid]
           + [(_load(42, 8), P(inv_a, p, g2, b))
              for p in range(2) for b in range(8) for g2 in range(4)])

    placed = _place([j[1] for j in jobs], [j[0] for j in jobs], streams)
    for v in range(16):
        latest[:] = [norm_rows(v)[8:]]
    for (_, _, before, fn, behind), tasks in zip(jobs, placed):
        for step in before:
            step()
        fn(tasks)
        for step in behind:
            step()
    for copy in o_cp.values():
        copy.wait()


@jax.jit
def pallas_recurrent_scan__spectral_gfnet__mixer_gmlp__prompt_kernel(
    A_x: jax.Array,
    A_w_r: jax.Array,
    A_w_i: jax.Array,
    B_x: jax.Array,
    B_w_in: jax.Array,
    B_w_sp: jax.Array,
    B_b_sp: jax.Array,
    B_w_out: jax.Array,
):
    del B_x
    args = (A_x.reshape(S, D), A_w_r.T, A_w_i.T, B_w_in.T, B_w_sp, B_b_sp.reshape(16, 128),
            B_w_out, *_constants())

    def buf(rows, cols, dtype):
        return pltpu.VMEM((rows + 8, cols), dtype)

    scratch = [pltpu.VMEM(a.shape, a.dtype) for a in args] + [
        buf(FH // 2, 7 * 256, U32),
        buf(7 * 128, F1, U32),
        [buf(128, D, U32)] * NB,
        [buf(64, 7 * 256, U32)] * (NB - 2),
        [buf(128, D, U32)] * NB,
        [buf(FH, 128, F32)] * (2 * NB),
        [buf(FQ // 2, 50 * 128, U32)] * 4,
        [buf(64, 46 * 128, U32)] * 12,
        [buf(F1, 7 * 256, F32)] * 4,
        [buf(F1 // 2, 8 * 128, U32)] * NB,
        [buf(128, D, F32)] * (2 * NB),
        [buf(S, 256, F32)] * 4,
        [pltpu.VMEM((2320, 128), F32)] * 8,
        [buf(128, D, U32)] * NB,
        buf(S, 256, U32),
        pltpu.VMEM((S, D), BF16),
        pltpu.SemaphoreType.DMA((10,)),
        pltpu.SemaphoreType.DMA(()),
    ]
    out = pl.pallas_call(
        _kernel,
        out_shape=jax.ShapeDtypeStruct((S, D), BF16),
        in_specs=[pl.BlockSpec(memory_space=pltpu.SMEM)]
        + [pl.BlockSpec(memory_space=pltpu.HBM)] * len(args),
        out_specs=pl.BlockSpec(memory_space=pltpu.HBM),
        scratch_shapes=scratch,
        compiler_params=pltpu.CompilerParams(
            vmem_limit_bytes=120 * 2 ** 20,
            flags={'XLA_TPU_RESCHEDULE_DMA_DONES': True}),
    )(np.zeros((1,), np.int32), *args)
    return out.reshape(1, S, D)
```

```python
import functools
import math

import numpy as np
import jax
import jax.numpy as jnp
from jax import lax
import jax.experimental.pallas as pl
import jax.experimental.pallas.tpu as pltpu

F32 = jnp.float32
BF16 = jnp.bfloat16
U32 = jnp.uint32
I32 = jnp.int32
NN = (((1,), (0,)), ((), ()))
NT = (((1,), (1,)), ((), ()))

S, D, FH = 2048, 512, 688
NB = S // 256
F0, F1 = 336, 352
FQ = F1 // 2
EPS = 1e-5

ALPHA = (math.sqrt(2.0 / math.pi) * 0.044715) ** (1.0 / 3.0)
GC = math.sqrt(2.0 / math.pi) / ALPHA
BETA = 0.5 / ALPHA

H_AT = ((6, 3), (7, 1))
TAIL = 'B0 B1 B2 B3 B4 I0 B5 I1 I2 I3 B6 I4 I5 I6 I7 B7'
Z0_AT = ('P', 4, 0)
Z1_AT = ('U', 4, 1)
Z3_AT = ('H', 0, 3, 4)
FOLD_AT = ('H', 0, 6, 0)
MIDDLE = ('H', 0, 1, 0)
LATE = ('Q', 1, 4, 3)
FILTER_AT = ('Q', 2, 0, 4)
WOUT_AT = ('Q', 2, 3, 0)
MARGIN = 340
PIN = 250
W_OPS = 0.5
HOLD_NORM, HOLD_PAIR, HOLD_FOLD, HOLD_WSP = (0, 2), ((0, 1), (2, 3)), (0, 1), (0, 3)


def _pack(m):
    u = np.asarray(m).astype(jnp.bfloat16).view(np.uint16).astype(np.uint32)
    return u[..., 0::2, :] | (u[..., 1::2, :] << 16)


def _constants():
    lane = np.arange(128)
    fwd, inv = [], []
    for k in (2 * lane, 2 * lane + 1):
        phi = 2.0 * np.pi * np.outer(lane - 127.5, k) / D
        weight = np.where(k == 0, 1.0, 2.0) / (D * S)
        fwd += [np.cos(phi) / ALPHA, -np.sin(phi) / ALPHA]
        inv += [(np.cos(phi) * weight).T, (-np.sin(phi) * weight).T.copy()]
    fwd[1][:, 0] = (-1.0) ** lane / ALPHA
    inv[1][0, :] = (-1.0) ** lane / (D * S)

    t = np.exp(-2j * np.pi * np.outer(np.arange(1, 8), np.arange(256)).reshape(-1, 1) / S)
    twid = np.concatenate([np.tile(t.real, (1, 128)), np.tile(t.imag, (1, 128))], axis=1)

    r = np.arange(16)
    f16 = np.exp(-2j * np.pi * np.outer(r, r) / 16)
    f128 = np.exp(-2j * np.pi * np.outer(lane, lane) / 128)
    nq = np.zeros((3, 128, 128))
    nq[0], nq[1] = f128.real, f128.imag
    m = np.block([[f16.real, -f16.imag], [f16.imag, f16.real]])
    nq[2, 0:32, 0:32] = m
    nq[2, 32:64, 0:32] = m.T
    tw = np.exp(-2j * np.pi * np.outer(r, lane) / S)
    tw = np.concatenate([tw.real, tw.imag])
    return _pack(np.stack(fwd + inv)), twid.astype(np.float32), _pack(nq), tw.astype(np.float32)


def _as_bf16(v):
    return pltpu.bitcast(v, BF16)


def _as_u32(v):
    return pltpu.bitcast(v.astype(BF16), U32)


def _cat0(xs):
    return jnp.concatenate(list(xs), axis=0)


def _cat1(xs):
    return jnp.concatenate(list(xs), axis=1)


def _tiles(v):
    return [v[:, 128 * j:128 * (j + 1)] for j in range(v.shape[1] // 128)]


def _groups(v):
    return [v[8 * g:8 * g + 8] for g in range(v.shape[0] // 8)]


def _rev_lanes(v):
    return jnp.take_along_axis(v, 127 - lax.broadcasted_iota(I32, v.shape, 1), axis=1)


def _gelu_core(u):
    return u + u * jnp.tanh(u * (GC + u * u))


def _rotate(z, num, den, sign):
    re, im = z
    num = (sign * num) % den
    if num == 0:
        return re, im
    if 4 * num == den:
        return -im, re
    if 2 * num == den:
        return -re, -im
    if 4 * num == 3 * den:
        return im, -re
    c = math.cos(2.0 * math.pi * num / den)
    s = math.sin(2.0 * math.pi * num / den)
    if (8 * num) % den == 0:
        if c * s > 0:
            return (re - im) * c, (re + im) * c
        return (re + im) * c, (im - re) * c
    return re * c - im * s, re * s + im * c


def _dft4(z, sign):
    (ar, ai), (br, bi), (cr, ci), (dr, di) = z
    pr, pi, qr, qi = ar + cr, ai + ci, ar - cr, ai - ci
    rr, ri, tr, ti = br + dr, bi + di, br - dr, bi - di
    o1, o3 = (qr + ti, qi - tr), (qr - ti, qi + tr)
    if sign > 0:
        o1, o3 = o3, o1
    return [(pr + rr, pi + ri), o1, (pr - rr, pi - ri), o3]


def _dft8_join(even, odd, j, sign):
    er, ei = even[j]
    if j == 2:
        tr, ti = odd[j]
        lo, hi = (er + ti, ei - tr), (er - ti, ei + tr)
        return (hi, lo) if sign > 0 else (lo, hi)
    tr, ti = _rotate(odd[j], j, 8, sign)
    return (er + tr, ei + ti), (er - tr, ei - ti)


SHORT = (2, 5, 6)


def _lhs_operand(k, a11, a12, a21, a22):
    if k == 0:
        return a21 + a22
    if k == 4:
        return a22
    if a11 is None:
        return {1: a22, 3: a21}.get(k)
    if k == 1:
        return a11 + a22
    if k == 3:
        return a21 - a11
    if k == 5:
        return a11 + a12
    return a11 if k == 2 else a12 - a22


def _rhs_operand(k, b11, b12, b21, b22):
    if k in (0, 5):
        return b22 if k else b11
    if k in (1, 3):
        return b11 + (b22 if k == 1 else b12)
    if k == 2:
        return b12 - b22
    return b21 - b11 if k == 4 else b21 + b22


def _load(ops, stores):
    return ops * W_OPS + stores


def _place(loads, cycles, streams):
    loads = np.array(loads, float)
    cycles = np.array(cycles, float)
    placed = [[] for _ in loads]
    order = sorted(range(len(streams)),
                   key=lambda n: (not streams[n][3], cycles[streams[n][0]:streams[n][1]].sum(), n))
    for n in order:
        first, last, tasks, even = streams[n]
        cost = np.array([c for c, _ in tasks], float)
        span = slice(first, last)
        lo, hi = 0.0, 8.0
        for _ in range(40):
            level = 0.5 * (lo + hi)
            if np.maximum(level * cycles[span] - loads[span], 0.0).sum() < cost.sum():
                lo = level
            else:
                hi = level
        share = np.maximum(hi * cycles[span] - loads[span], 0.0)
        if even:
            share = cycles[span] * (cost.sum() / cycles[span].sum())
        where = first + np.searchsorted(np.cumsum(share), np.cumsum(cost) - 0.5 * cost)
        np.add.at(loads, where, cost)
        for j in np.unique(where):
            mine = [t for t, at in zip(tasks, where) if at == j]
            placed[j] += [((m + 0.5) / len(mine), n, t) for m, t in enumerate(mine)]
    return [[t for _, _, t in sorted(p, key=lambda e: e[:2])] for p in placed]


def _kernel(zero_s, x_hbm, wr_hbm, wi_hbm, win_hbm, wsp_hbm, b_hbm, wout_hbm,
            dmat_hbm, twid_hbm, nq_hbm, tw_hbm, o_hbm,
            x_v, wr_v, wi_v, win_v, wsp_v, b_v, wout_v, dmat_v, twid_v, nq_v, tw_v,
            wis_v, wos_v, xn_v, xs_v, ep_v, act_v, zs_v, ws_v, prod_v, hs_v, gate_v, zf, zp,
            yo_v, wt_v, col_v, o_v, sem_i, sem_o):
    P = functools.partial
    zero = zero_s[0]
    sealed = set()

    def fetch(ref, r0, r1, c0=0, c1=None, use=0):
        if (id(ref), use) not in sealed:
            sealed.add((id(ref), use))
            last = ref.shape[0] // 8 - 1
            spare = pl.multiple_of(8 * jnp.clip(zero + last, 0, last), 8)
            ref[pl.ds(spare, 8), 0:128] = jnp.zeros((8, 128), ref.dtype)
        return ref[r0:r1, c0:c1]

    def part(src, dst, *idx):
        return src.at[idx], dst.at[idx]

    stages = [
        [part(x_hbm, x_v, slice(0, 256))],
        [part(win_hbm, win_v, slice(FH, FH + F0))],
        [part(x_hbm, x_v, slice(256, 384))],
        [part(x_hbm, x_v, slice(384, 512))],
        [part(win_hbm, win_v, slice(FH + F0, FH + 512))],
        [part(win_hbm, win_v, slice(FH + 512, 2 * FH))],
        [part(win_hbm, win_v, slice(0, F0))],
        [part(win_hbm, win_v, slice(F0, FH)), part(x_hbm, x_v, slice(512, 768))],
        [part(x_hbm, x_v, slice(768, 1280))],
        [part(x_hbm, x_v, slice(1280, S)), part(wsp_hbm, wsp_v, slice(0, 512), slice(0, 1024))],
        [part(wsp_hbm, wsp_v, slice(0, 512), slice(1024, S)),
         part(wsp_hbm, wsp_v, slice(512, 1024)), (b_hbm, b_v), (dmat_hbm, dmat_v),
         part(wsp_hbm, wsp_v, slice(1024, 1536), slice(0, 1024))],
        [(wr_hbm, wr_v), (wi_hbm, wi_v), (twid_hbm, twid_v), (nq_hbm, nq_v), (tw_hbm, tw_v),
         part(wsp_hbm, wsp_v, slice(1024, 1536), slice(1024, S)),
         part(wsp_hbm, wsp_v, slice(1536, S)), (wout_hbm, wout_v)],
    ]
    for n, stage in enumerate(stages):
        for src, dst in stage:
            pltpu.make_async_copy(src, dst, sem_i.at[n]).start()
    latest = []

    def arrive(n):
        slot = n
        if latest:
            held_zero = after(latest[0], jnp.zeros((8, 128), I32))[0, 0]
            slot = jnp.clip(n + held_zero, 0, len(stages) - 1)
        for src, dst in stages[n]:
            pltpu.make_async_copy(src, dst, sem_i.at[slot]).wait()

    edges = sorted(list(range(0, S + 1, 128)) + [S - 192, S - 160])
    o_cp = {b: pltpu.make_async_copy(o_v.at[a:b], o_hbm.at[a:b], sem_o)
            for a, b in zip(edges, edges[1:])}

    lane = lax.broadcasted_iota(I32, (1, 128), 1)
    arrive(0)
    never = jnp.full((8, 128), zero, I32) > 0

    def after(dep, v):
        if dep is None:
            return v
        if v.dtype != dep.dtype:
            dep = pltpu.bitcast(dep, v.dtype)
        return _cat0(jnp.where(never, dep, g) for g in _groups(v))

    def widen(dep, packed, hold=(0,)):
        return _as_bf16(_cat1(after(dep if n in hold else None, t)
                              for n, t in enumerate(_tiles(packed)))).astype(F32)

    def matmuls(pairs, dims, tasks):
        res = [lax.dot_general(_as_bf16(a), _as_bf16(b), dims, preferred_element_type=F32)
               for a, b in pairs]
        slots = [(n, c) for n, (a, _) in enumerate(pairs) for c in range(0, a.shape[1], 128)]
        ends = {m // 4: n for m, (n, c) in enumerate(slots) if c + 128 >= pairs[n][0].shape[1]}
        g = max(res[0].shape[0] - PIN, 0) // 8
        latest[:] = [res[0][8 * g:8 * g + 8]]
        start, total = 0.0, sum(cost for cost, _ in tasks)
        for cost, task in tasks:
            at = -(-len(slots) // 4) * start / total
            r = res[ends[min(k for k in ends if k >= int(at))]]
            g = int((at - int(at)) * (r.shape[0] // 8))
            task(r[8 * g:8 * g + 8])
            start += cost
        return res

    pre, stat = {}, {}

    def xn_rows(j, r=0):
        return (xn_v[j], r) if j < 4 else (xn_v[2 + j // 2], 64 * (j % 2) + r)

    def norm_rows(v, dep=None):
        packed = pltpu.bitcast(x_v[16 * v:16 * v + 16, :], U32)
        x0, x1, x2, x3 = _tiles(widen(dep, packed, HOLD_NORM))
        mean = jnp.sum((x0 + x1) + (x2 + x3), axis=1, keepdims=True) * (1.0 / D)
        sq = jnp.sum((x0 * x0 + x1 * x1) + (x2 * x2 + x3 * x3), axis=1, keepdims=True)
        var = jnp.maximum(sq * (1.0 / D) - mean * mean, 0.0)
        scale = lax.rsqrt(var + EPS) * ALPHA
        xn = [(a - mean) * scale for a in (x0, x1, x2, x3)]
        ref, r = xn_rows(v // 8, 8 * (v % 8))
        ref[r:r + 8, :] = _as_u32(_cat1(xn))
        return xn[3]

    def xn_operands(i, v, dep):
        a, b = (widen(dep, xn_v[2 + i][r:r + 8, :], HOLD_PAIR[r // 64])
                for r in (8 * v, 64 + 8 * v))
        for k in (1, 2, 3, 4, 6):
            xs_v[i - 2][8 * v:8 * v + 8, 256 * k:256 * (k + 1)] = _as_u32(
                _rhs_operand(k, a[:, :256], b[:, :256], a[:, 256:], b[:, 256:]))

    def norm_tasks(i):
        rows = [(_load(72, 6), P(norm_rows, 16 * i + 8 * h + v))
                for v in range(8) for h in range(2)]
        tasks = rows[:4]
        for v in range(8):
            tasks += rows[4 + 2 * v:6 + 2 * v] + [(_load(55, 11), P(xn_operands, i, v))]
        return tasks

    def win_operands(v, dep):
        a, b = (widen(dep, pltpu.bitcast(win_v[r:r + 16, :], U32), HOLD_PAIR[r // FH])
                for r in (16 * v, FH + 16 * v))
        for k in range(7):
            wis_v[8 * v:8 * v + 8, 256 * k:256 * (k + 1)] = _as_u32(
                _lhs_operand(k, a[:, :256], a[:, 256:], b[:, :256], b[:, 256:]))

    def activate(j, r0, u):
        a = _gelu_core(u)
        act_v[j][r0:r0 + u.shape[0], :] = a
        for g in _groups(a):
            stat[j] = (stat[j][0] + g, stat[j][1] + g * g) if j in stat else (g, g * g)
        if r0 + u.shape[0] == FH:
            m = jnp.sum(stat[j][0], axis=0, keepdims=True) * (1.0 / FH)
            v = jnp.sum(stat[j][1], axis=0, keepdims=True) * (1.0 / FH) - m * m
            r = lax.rsqrt(jnp.maximum(v, 0.0) + EPS / BETA ** 2) * (0.5 * BETA)
            stat[j] = (jnp.broadcast_to(m, (8, 128)), jnp.broadcast_to(r, (8, 128)))

    def plain_job(half, j, r0, r1, tasks):
        w = pltpu.bitcast(win_v[FH * half + r0:FH * half + r1, :], U32)
        u, = matmuls([(w, fetch(xn_v[j], 0, 64))], NT, tasks)
        if half:
            activate(j, r0, u)
        else:
            pre.setdefault(('u', j), []).extend(_groups(u))

    def project_job(i, n, tasks):
        def pair(k, r0=0, r1=FH // 2):
            if k in (0, 5):
                h = k // 5
                rhs = fetch(xn_v[2 + i], 64 * h, 64 * (h + 1), 256 * h, 256 * (h + 1))
            else:
                rhs = fetch(xs_v[i - 2], 0, 64, 256 * k, 256 * (k + 1))
            return fetch(wis_v, r0, r1, 256 * k, 256 * (k + 1)), rhs
        m = pre.setdefault(('m', i), [])
        if n < 3:
            m += matmuls([pair(2 * n), pair(2 * n + 1)], NT, tasks)
        else:
            m.append(_cat0(matmuls([pair(6, 0, F1 // 2), pair(6, F1 // 2)], NT, tasks)))
        if n == 1:
            activate(2 * i + 1, 0, (m[1] - m[0]) + (m[2] + m[3]))
        if n == 2:
            activate(2 * i, 0, m[0] + m[4])

    def linear1(t, w):
        if ('m', t) not in pre:
            return (_cat0(pre['u', j][2 * w:2 * w + 2]) for j in (2 * t, 2 * t + 1))
        m1, m3, m4, m5, m7 = (pre['m', t][k][16 * w:16 * w + 16] for k in (1, 2, 4, 5, 6))
        return (m1 + m4) + (m7 - m5), m3 + m5

    z_order = ((2, (0,)), (4, (3,)), (1, ()), (0, (2,)), (3, ()), (5, (1,)), (6, ()))
    w_order = ((0, (0,)), (5, (3,)), (1, ()), (2, (1,)), (3, ()), (4, (2,)), (6, ()))
    w_plain = ((0, 0), (0, 5), (5, 0), (5, 5))

    def slots_of(order, skip):
        keys = [(k, j) for k, _ in order for j in range(7) if (k, j) not in skip]
        return {key: n for n, key in enumerate(keys)}
    z_slots, w_slots = slots_of(z_order, ()), slots_of(w_order, w_plain)

    def nested_operands(ref, v, source, rule, order, slots):
        state = {'left': ()}

        def step(k, fresh, dep):
            for n in fresh:
                state[n] = source(n, dep)
            blocks = [rule(k, *(state[n][m] if n in state else None for n in range(4)))
                      for m in range(4)]
            if not fresh:
                blocks[3] = _cat0([blocks[3][:8], after(dep, blocks[3][8:])])
            js = [j for j in range(7) if (k, j) in slots]
            ops = [rule(j, *blocks) for j in js]
            ops = tuple(blocks[3] if op is None else op for op in ops)
            n0 = slots[k, js[0]] - len(state['left'])
            ops = state['left'] + ops + (ops[-1:] if k == 6 else ())
            for n in range(0, len(ops) - 1, 2):
                ref[8 * v:8 * v + 8, 128 * (n0 + n):128 * (n0 + n + 2)] = _as_u32(
                    _cat1(ops[n:n + 2]))
            state['left'] = ops[len(ops) // 2 * 2:]
        return [(0.8 * _load(27 + 14 * len(fresh), 7 + 5 * len(fresh)), P(step, k, fresh))
                for k, fresh in order]

    def z2_tasks(q):
        def source(v, n, dep):
            tiles = (4 * q + n % 2, 4 * q + 2 + n % 2)
            mean = {j: after(dep, stat[j][0]) for j in tiles}

            def normed(j, r):
                if n < 2 and r >= F0:
                    return None
                r += F0 * (n // 2)
                return _cat0((a - mean[j]) * stat[j][1]
                             for a in _groups(fetch(act_v[j], r, r + 16)))
            return [normed(j, r) for r in (FQ + 16 * v, 16 * v) for j in tiles]
        return [t for v in range(FQ // 16) for t in nested_operands(
            zs_v[q], v, P(source, v), _lhs_operand, z_order, z_slots)]

    def wsp_tile(r, c, rows):
        return pltpu.bitcast(wsp_v[r:r + rows, c:c + 128], U32)

    def wsp_tasks(tq, qs):
        def source(q, v, n, dep):
            return [widen(dep if m in HOLD_WSP else None,
                          wsp_tile(512 * tq + 256 * (m % 2) + 128 * (n % 2) + 16 * v,
                                   512 * q + 256 * (m // 2) + 128 * (n // 2), 16))
                    for m in range(4)]
        return [t for q in qs for v in range(8) for t in nested_operands(
            ws_v[4 * (tq % 3) + q], v, P(source, q, v), _rhs_operand, w_order, w_slots)]

    inner = {}

    def height(k, j):
        return FQ - 16 if k in SHORT and j in SHORT else FQ

    def product_job(tq, k, js, qs, tasks):
        def pair(j, r0=0, r1=None):
            c = 128 * z_slots[k, j]
            lhs = _cat1(fetch(zs_v[q], r0, r1 or height(k, j) // 2, c, c + 128) for q in qs)
            if (k, j) in w_plain:
                o = 256 * (j // 5) + 128 * (k // 5)
                return lhs, _cat1(wsp_tile(512 * tq + o, 512 * q + o, 128) for q in qs)
            c = 128 * w_slots[k, j]
            return lhs, _cat1(fetch(ws_v[4 * (tq % 3) + q], 0, 64, c, c + 128, tq) for q in qs)
        if len(js) * len(qs) == 4:
            res = matmuls([pair(j) for j in js], NT, tasks)
        else:
            res = [_cat0(matmuls([pair(js[0], 0, 48), pair(js[0], 48)], NT, tasks))]
        for j, r in zip(js, res):
            inner[tq, k, j] = inner[tq, k, j] + r if (tq, k, j) in inner else r
        if qs[-1] == 3:
            out, n = prod_v[tq], height(k, 2)
            m2, m1, m3, m6, m4, m5, m7 = (inner.get((tq, k, j)) for j in range(7))
            c0, c1 = slice(256 * k, 256 * k + 128), slice(256 * k + 128, 256 * k + 256)
            if 3 in js:
                c22 = (m1 - m2) + m6
                out[0:FQ, c1] = _cat0([c22[:n] + m3, c22[n:]]) if n < FQ else c22 + m3
            if 4 in js:
                out[0:FQ, c0] = m2 + m4
            if 5 in js:
                out[FQ:FQ + n, c1] = m3 + m5
            if 6 in js:
                out[FQ:FQ + n, c0] = (m1[:n] + m4[:n]) + (m7 - m5)

    def gate_tasks(t, v):
        state = {}

        def bias(j, dep):
            b = after(dep, jnp.broadcast_to(b_v[j:j + 1, :].astype(F32) * (0.5 * BETA), (8, 128)))
            return _cat0([b, b])

        def outer(k):
            c = 256 * k + 128 * (t % 2)
            return fetch(prod_v[t // 2], 16 * v, 16 * v + 16, c, c + 128)

        def lower(dep):
            m2, m1, m6, m4 = (outer(k) for k in (0, 1, 3, 4))
            m4 = m4 + bias(2 * t, dep)
            m3 = bias(2 * t + 1, dep)
            if 16 * v < F0:
                m3 = m3 + outer(2)
            z21, z22 = (_gelu_core(after(dep, u)) for u in linear1(t, F0 // 16 + v))
            state['v'] = (m1 + m4, m3, z21 * (m2 + m4), z22 * ((m1 - m2) + (m3 + m6)))

        def upper(dep):
            m14, m3, h21, h22 = state['v']
            if 16 * v < F0:
                m5, m7 = outer(5), outer(6)
                z11, z12 = (_gelu_core(after(dep, u)) for u in linear1(t, v))
                h11, h12 = z11 * (m14 + (m7 - m5)), z12 * (m3 + m5)
                ops = [_rhs_operand(k, h11, h12, h21, h22) for k in range(7)]
            else:
                ops = [h22, h22, h22, h22, h21, h22, h21 + h22]
            hs_v[t][8 * v:8 * v + 8, :] = _as_u32(_cat1(ops + [h22]))
        return [(_load(52, 3), lower), (_load(62, 9), upper)]

    def fold_rows(b, n, dep):
        ref, r = xn_rows(4 * (n % 4) + b // 2, 32 * (b % 2) + 8 * (n // 4))
        x0, x1, x2, x3 = _tiles(widen(dep, fetch(ref, r, r + 8), HOLD_FOLD))
        s02, d02, s13, d13 = x0 + x2, x0 - x2, _rev_lanes(x1 + x3), _rev_lanes(x1 - x3)
        ep_v[b][8 * n:8 * n + 8, :] = _as_u32(_cat1([s02 + s13, s02 - s13, d02 + d13, d02 - d13]))

    def get(stage, p, n):
        return tuple(_tiles(fetch(zf[2 * (stage % 2) + p], 8 * n, 8 * n + 8, use=stage)))

    def put(stage, p, n, z):
        zf[2 * (stage % 2) + p][8 * n:8 * n + 8, :] = _cat1(z)

    def gather(cols, shifts):
        for shift in shifts:
            cols = [jnp.where(lane & shift != 0, pltpu.roll(hi, shift, 1), lo)
                    for lo, hi in zip(cols[0::2], cols[1::2])]
        return cols[0]

    def dft_job(b, tasks):
        res = matmuls([(fetch(ep_v[b], 0, 128, 128 * j, 128 * (j + 1)), dmat_v[j])
                       for j in range(4)], NN, tasks)
        col_v[16 * b:16 * b + 16, :] = gather(
            [res[1][r:r + 16] for r in range(0, 256, 16)], (32, 64, 1, 2))
        res[1] = jnp.where(lane == 0, 0.0, res[1])
        for g in range(8):
            for p in range(2):
                rows = [64 * (g // 2) + 16 * a + 8 * (g % 2) for a in range(4)]
                t = _dft4([(res[2 * p][r:r + 8], res[2 * p + 1][r:r + 8]) for r in rows], -1)
                for c in range(4):
                    put(0, p, 8 * (8 * c + b) + g, _rotate(t[c], b * c, 32, -1))

    def weight_rows(j, c, dep):
        t = pltpu.bitcast((wr_v, wi_v)[c][0:256, 128 * j:128 * (j + 1)], U32)
        wt_v[128 * j:128 * (j + 1), 128 * c:128 * (c + 1)] = _cat0([after(dep, t[:8]), t[8:]]).T

    def held(dep, z):
        return [(after(dep, z[0][0]), z[0][1])] + z[1:]

    def radix8(source, sink, sign, ops, stores):
        def dft8(dep):
            even, odd = ([source(n) for n in range(h, 8, 2)] for h in range(2))
            even, odd = _dft4(even[:2] + held(dep, even[2:]), sign), _dft4(odd, sign)
            for j in range(4):
                for n, z in zip((j, j + 4), _dft8_join(even, odd, j, sign)):
                    sink(n, z)
        return _load(56 + ops, stores), dft8

    def fwd_b(p, g, c):
        return radix8(lambda b: get(0, p, 8 * (8 * c + b) + g),
                      lambda e, z: put(1, p, 8 * (c + 4 * e) + g,
                                       _rotate(z, (c + 4 * e) * g, 256, -1)), -1, 42, 16)

    def fwd_g(p, k):
        def sink(m, z):
            r = 9 * (k + 32 * m)
            zp[2 * p][r:r + 8, :], zp[2 * p + 1][r:r + 8, :] = z
        return radix8(lambda g: get(1, p, 8 * k + g), sink, -1, 0, 16)

    def filter_tasks(p, w):
        spectrum = {}

        def twiddle(i):
            r = 256 * (i - 1) + 8 * w
            return twid_v[r:r + 8, 0:128], twid_v[r:r + 8, 128:256]

        def source(i):
            re, im = (zp[2 * p + h][pl.ds(72 * w + i, 8, stride=9), :] for h in range(2))
            if i == 0:
                return re, im
            tr, ti = twiddle(i)
            return re * tr - im * ti, re * ti + im * tr

        def weigh(dep):
            arg = after(dep, jnp.full((8, 128), 0xFFFF0000 if p else 16, U32))
            for n in range(8):
                (re, im), r = spectrum[n], 256 * n + 8 * w
                wr, wi = (pltpu.bitcast(u & arg if p else u << arg, F32)
                          for u in _tiles(fetch(wt_v, r, r + 8)))
                spectrum[n] = (re * wr - im * wi, re * wi + im * wr)

        def sink(i, z):
            re, im = z
            if i:
                tr, ti = twiddle(i)
                re, im = re * tr + im * ti, im * tr - re * ti
            rows = pl.ds(72 * w + i, 8, stride=9)
            zp[4 + 2 * p][rows, :], zp[5 + 2 * p][rows, :] = re, im
        return [radix8(source, lambda n, z: spectrum.update({n: z}), -1, 42, 2),
                (_load(65, 2), weigh), radix8(lambda n: spectrum[n], sink, 1, 42, 16)]

    def inv_g(p, k):
        def source(m):
            r = 9 * (k + 32 * m)
            return zp[4 + 2 * p][r:r + 8, :], zp[5 + 2 * p][r:r + 8, :]
        return radix8(source, lambda g, z: put(2, p, 8 * k + g, _rotate(z, k * g, 256, 1)),
                      1, 42, 16)

    def inv_b(p, g, c):
        return radix8(lambda e: get(2, p, 8 * (c + 4 * e) + g),
                      lambda b, z: put(3, p, 8 * (c + 4 * b) + g, _rotate(z, b * c, 32, 1)),
                      1, 29, 16)

    def inv_a(p, g2, b, dep):
        t = [_dft4(held(dep, [get(3, p, 8 * (c + 4 * b) + g) for c in range(4)]), 1)
             for g in (2 * g2, 2 * g2 + 1)]
        r = 32 * (b % 4) + 8 * g2
        for a in range(4):
            yo_v[2 * a + b // 4][r:r + 8, 256 * p:256 * (p + 1)] = _as_u32(
                _cat0([_cat1(t[0][a]), _cat1(t[1][a])]))

    def nyquist():
        def mm(a, b):
            return jnp.dot(a.astype(BF16), b.astype(BF16), preferred_element_type=F32)
        sub = lax.broadcasted_iota(I32, (16, 128), 0)
        cr, ci = tw_v[0:16, :], tw_v[16:32, :]
        pad = jnp.zeros((96, 128), F32)
        col = gather([fetch(col_v, r, r + 16) for r in range(0, 128, 16)], (4, 8, 16))
        tr, ti = mm(col, _as_bf16(nq_v[0])), mm(col, _as_bf16(nq_v[1]))
        yield
        xf = mm(_as_bf16(nq_v[2, 0:16, :]), _cat0([tr * cr - ti * ci, tr * ci + ti * cr, pad]))
        xr, xi = xf[:16], xf[16:]
        yield
        wn = []
        for ref in (wr_v, wi_v):
            acc = jnp.zeros((16, 128), F32)
            for j, piece in enumerate(_tiles(ref[256:257, :].astype(F32))):
                acc = jnp.where(sub == j, piece, acc)
            wn.append(acc)
        u = mm(_as_bf16(nq_v[2, 16:32, :]),
               _cat0([xr * wn[0] - xi * wn[1], xr * wn[1] + xi * wn[0], pad]))
        ur, ui = u[:16], u[16:]
        yield
        proj['n'] = _as_u32(mm(ur * cr + ui * ci, _as_bf16(nq_v[0]))
                            + mm(ui * cr - ur * ci, _as_bf16(nq_v[1])))
        yield

    depth = (F0, F1, F0, F0, F1, F1, F1)
    proj = {}

    def wout_operand(k, dep):
        lo = _cat0([wout_v[0:F0, :].astype(F32), jnp.zeros((F1 - F0, D), F32)])
        hi = wout_v[F0:FH, :].astype(F32)
        op = _lhs_operand(k, lo[:, :256], hi[:, :256], lo[:, 256:], hi[:, 256:])
        wos_v[128 * k:128 * (k + 1), 0:depth[k]] = pltpu.bitcast(
            op[0:depth[k]].astype(BF16).T, U32)

    def emit(i, h):
        if ('y', i) not in proj or (i, 6) not in proj:
            return
        for r in range(128 * h, 128 * (h + 1), 16):
            e0, o0, e1, o1 = (a[r:r + 16] for a in proj['y', i])
            lo0, hi0, lo1, hi1 = e0 + o0, e0 - o0, e1 + o1, e1 - o1
            s = _cat1([lo0 + lo1, _rev_lanes(hi0 + hi1), lo0 - lo1, _rev_lanes(hi0 - hi1)])
            g = fetch(gate_v[2 * i + h], r % 128, r % 128 + 16)
            rows = slice(256 * i + r, 256 * i + r + 16)
            o_v[rows, :] = (x_v[rows, :].astype(F32) + s * g).astype(BF16)
            if rows.stop in o_cp:
                o_cp[rows.stop].start()

    def output_job(i, ks, tasks):
        res = matmuls([(fetch(wos_v, 128 * k, 128 * (k + 1), 0, depth[k]),
                        fetch(hs_v[i], 0, depth[k] // 2, 128 * k, 128 * (k + 1))) for k in ks],
                      NN, tasks)
        proj.update({(i, k): r for k, r in zip(ks, res)})

        def keep(h, c, b):
            gate_v[2 * i + h][0:128, 256 * c:256 * (c + 1)] = (b + b * jnp.tanh(b)).T
        m2, m1, m3, m6 = (proj[i, k] for k in range(4))
        if ks[0] == 0:
            keep(1, 1, (m1 - m2) + (m3 + m6))
        else:
            m5, m4, m7 = res
            keep(1, 0, m3 + m5)
            emit(i, 1)
            keep(0, 1, m2 + m4)
            keep(0, 0, (m1 + m4) + (m7 - m5))
            emit(i, 0)

    def inverse_job(i, tasks):
        y = _tiles(fetch(yo_v[i], 0, 128))
        col = _cat0(pltpu.roll(proj['n'], (128 - v) % 128, 1) for v in range(16 * i, 16 * (i + 1)))
        y[1] = jnp.where(lane == 0, col, y[1])
        proj['y', i] = matmuls([(y[j], dmat_v[4 + j]) for j in range(4)], NN, tasks)
        emit(i, 0)
        emit(i, 1)

    jobs, names, streams = [], {}, []

    def job(name, cycles, load, fn):
        names[name] = len(jobs)
        jobs.append((cycles, load, [], fn, []))

    def half_products(k, qs):
        for js in ((0, 1), (2, 3), (4, 5), (6,)):
            job(('H', qs[0], k, js[0]), 88 * len(js),
                _load(22 + 24 * qs[0], 22 + 3 * qs[0]) * len(js), P(product_job, 0, k, js, qs))

    def stream(first, last, tasks, skip=0, margin=MARGIN, even=False):
        first, last, gap = names[first] + skip, names[last], 0
        while gap < margin and last - 1 > first:
            last -= 1
            gap += jobs[last][0]
        streams.append((first, last, tasks, even))

    for n, (half, r0, r1) in enumerate(((1, 0, F0), (1, F0, 512), (1, 512, FH), (0, 0, F0),
                                        (0, F0, FH))):
        for j in range(4):
            job(('P', n, j), r1 - r0, _load(215 + 344 * half, 43), P(plain_job, half, j, r0, r1))
    for i in range(2, NB):
        for n, load in enumerate(((172, 172), (1118, 172), (946, 258), (86, 86))):
            job(('U', i, n), FH if n < 3 else FH // 2, _load(*load), P(project_job, i, n))
            if (i, n) in H_AT:
                half_products(H_AT.index((i, n)), (0, 1))
    for k in range(len(H_AT), 7):
        half_products(k, (0, 1))
    for k in range(7):
        half_products(k, (2, 3))
        job(('D', k), 256, _load(500, 140), P(dft_job, k))
    for tq in range(1, 4):
        for k in range(7):
            for j in range(7):
                job(('Q', tq, k, j), height(k, j), _load(91, 28),
                    P(product_job, tq, k, (j,), range(4)))
            if (tq, k) == (1, 0):
                job(('D', 7), 256, _load(500, 140), P(dft_job, 7))
    for kind, i in ((a, int(b)) for a, b in TAIL.split()):
        if kind == 'B':
            job(('B', i, 0), 768, 1.3 * _load(420, 128), P(output_job, i, (0, 1, 2, 3)))
            job(('B', i, 1), 576, 1.3 * _load(550, 160), P(output_job, i, (5, 4, 6)))
        else:
            job(('I', i), 256, _load(900, 100), P(inverse_job, i))

    for n, name in enumerate((('P', 0, 0), ('P', 0, 1), ('P', 0, 2), ('P', 1, 0), ('P', 2, 0),
                              ('P', 3, 0), ('P', 4, 0), ('U', 2, 0), ('U', 4, 0), MIDDLE, LATE)):
        jobs[names[name]][2].append(P(arrive, n + 1))
    for j in (2, 3):
        jobs[names['P', 0, j - 1]][2].extend(P(norm_rows, v) for v in range(8 * j, 8 * j + 8))
    steps = nyquist()
    for k in range(4):
        jobs[names['Q', 2, k, 3]][4].append(P(next, steps))

    ops = [(_load(66, 15), P(win_operands, v)) for v in range(FH // 16)]
    stream(('P', 3, 0), ('P', 4, 0), ops[:F0 // 16], margin=0)
    stream(('P', 4, 0), ('U', 2, 0), ops[F0 // 16:], margin=1)
    for i in range(2, NB):
        stream(('P', 4, 0) if i == 2 else ('U', i - 1, 0), ('U', i, 0), norm_tasks(i), margin=1)
    for b in range(8):
        stream(('D', b - 1) if b else FOLD_AT, ('D', b),
               [(_load(36, 5), P(fold_rows, b, n)) for n in range(16)], margin=170, even=True)
    stream(Z0_AT, Z1_AT, z2_tasks(0), margin=0)
    stream(Z1_AT, ('H', 0, 0, 0), z2_tasks(1) + wsp_tasks(0, (0, 1)))
    stream(('H', 0, 0, 0), MIDDLE, z2_tasks(2), margin=0)
    stream(MIDDLE, Z3_AT, wsp_tasks(0, (2, 3)), margin=0)
    stream(Z3_AT, ('H', 2, 0, 0), z2_tasks(3))
    stream(('H', 2, 0, 0), ('Q', 1, 0, 0), wsp_tasks(1, range(4)))
    stream(('Q', 1, 0, 0), LATE, wsp_tasks(2, (0, 1)), margin=0)
    stream(LATE, ('Q', 2, 0, 0), wsp_tasks(2, (2, 3)))
    stream(('Q', 2, 0, 0), ('Q', 3, 0, 0), wsp_tasks(3, range(4)))
    for t in range(NB):
        stream(('Q', t // 2, 6, 6) if t > 1 else ('H', 2, 6, 6), ('B', t, 0),
               [task for v in range(F1 // 16) for task in gate_tasks(t, v)], skip=3)
    stream(WOUT_AT, ('B', 0, 0), [(_load(250, 60), P(wout_operand, k)) for k in range(7)],
           even=True)
    grid = [(p, c, n) for p in range(2) for c in range(4) for n in range(8)]
    stream(('D', 7), FILTER_AT,
           [fwd_b(p, g, c) for p, c, g in grid] + [fwd_g(p, c + 4 * e) for p, c, e in grid],
           skip=1, margin=0)
    stream(LATE, FILTER_AT,
           [(_load(18, 16), P(weight_rows, j, c)) for j in range(16) for c in range(2)], even=True)
    stream(FILTER_AT, ('I', 0),
           [task for p, c, n in grid for task in filter_tasks(p, 8 * c + n)]
           + [inv_g(p, c + 4 * e) for p, c, e in grid] + [inv_b(p, g, c) for p, c, g in grid]
           + [(_load(42, 8), P(inv_a, p, g2, b))
              for p in range(2) for b in range(8) for g2 in range(4)])

    placed = _place([j[1] for j in jobs], [j[0] for j in jobs], streams)
    for v in range(16):
        latest[:] = [norm_rows(v)[8:]]
    for (_, _, before, fn, behind), tasks in zip(jobs, placed):
        for step in before:
            step()
        fn(tasks)
        for step in behind:
            step()
    for copy in o_cp.values():
        copy.wait()


@jax.jit
def pallas_recurrent_scan__spectral_gfnet__mixer_gmlp__prompt_kernel(
    A_x: jax.Array,
    A_w_r: jax.Array,
    A_w_i: jax.Array,
    B_x: jax.Array,
    B_w_in: jax.Array,
    B_w_sp: jax.Array,
    B_b_sp: jax.Array,
    B_w_out: jax.Array,
):
    del B_x
    args = (A_x.reshape(S, D), A_w_r.T, A_w_i.T, B_w_in.T, B_w_sp, B_b_sp.reshape(16, 128),
            B_w_out, *_constants())

    def buf(rows, cols, dtype):
        return pltpu.VMEM((rows + 8, cols), dtype)

    scratch = [pltpu.VMEM(a.shape, a.dtype) for a in args] + [
        buf(FH // 2, 7 * 256, U32),
        buf(7 * 128, F1, U32),
        [buf(64, D, U32)] * 4 + [buf(128, D, U32)] * (NB - 2),
        [buf(64, 7 * 256, U32)] * (NB - 2),
        [buf(128, D, U32)] * NB,
        [buf(FH, 128, F32)] * (2 * NB),
        [buf(FQ // 2, 50 * 128, U32)] * 4,
        [buf(64, 46 * 128, U32)] * 12,
        [buf(F1, 7 * 256, F32)] * 4,
        [buf(F1 // 2, 8 * 128, U32)] * NB,
        [buf(128, D, F32)] * (2 * NB),
        [buf(S, 256, F32)] * 4,
        [pltpu.VMEM((2320, 128), F32)] * 8,
        [buf(128, D, U32)] * NB,
        buf(S, 256, U32),
        buf(128, 128, F32),
        pltpu.VMEM((S, D), BF16),
        pltpu.SemaphoreType.DMA((12,)),
        pltpu.SemaphoreType.DMA(()),
    ]
    out = pl.pallas_call(
        _kernel,
        out_shape=jax.ShapeDtypeStruct((S, D), BF16),
        in_specs=[pl.BlockSpec(memory_space=pltpu.SMEM)]
        + [pl.BlockSpec(memory_space=pltpu.HBM)] * len(args),
        out_specs=pl.BlockSpec(memory_space=pltpu.HBM),
        scratch_shapes=scratch,
        compiler_params=pltpu.CompilerParams(
            vmem_limit_bytes=120 * 2 ** 20,
            flags={'XLA_TPU_RESCHEDULE_DMA_DONES': True}),
    )(np.zeros((1,), np.int32), *args)
    return out.reshape(1, S, D)
```
